```python
import os as _os
_os.environ.setdefault('JAX_PLATFORMS', 'cpu')
import jax
import jax.numpy as jnp

def _softmax(x, axis=-1):
    return jax.nn.softmax(x, axis=axis)

def _gelu(x):
    return jax.nn.gelu(x, approximate=True)

def _silu(x):
    return jax.nn.silu(x)

def _sigmoid(x):
    return jax.nn.sigmoid(x)

def _layernorm(x, axis=-1, eps=1e-05):
    m = jnp.mean(x, axis=axis, keepdims=True)
    v = jnp.var(x, axis=axis, keepdims=True)
    return (x - m) / jnp.sqrt(v + eps)

def _scatter_add(tgt, idx, src, axis=0):
    return tgt.at[idx].add(src)

def _segment_sum(src, seg, n):
    return jax.ops.segment_sum(src, seg, n)

class _Rng:

    def __init__(self, key):
        self._k = key

    def _next(self):
        self._k, sub = jax.random.split(self._k)
        return sub

    def normal(self, shape):
        return jax.random.normal(self._next(), shape, dtype=jnp.bfloat16)

    def randint(self, lo, hi, shape):
        return jax.random.randint(self._next(), shape, lo, hi, dtype=jnp.int32)

    def uniform(self, shape, lo=0.0, hi=1.0):
        return jax.random.uniform(self._next(), shape, jnp.bfloat16, lo, hi)

    def permutation(self, n):
        return jax.random.permutation(self._next(), n)
kernel_name = 'recurrent_scan__spectral_gfnet__mixer_gmlp__prompt'

def setup_inputs():
    _rng = _Rng(jax.random.key(int.from_bytes(__import__("os").urandom(4), "little")))
    _w = lambda a: (lambda t: t.astype(jnp.bfloat16) if jnp.issubdtype(t.dtype, jnp.floating) else t)(jnp.asarray(a))

    def _A_setup():
        B, S, D = (1, 2048, 512)
        Df = D // 2 + 1
        return {'x': _w((lambda *s: _rng.normal(s) * 0.05)(B, S, D)), 'w_r': _w((lambda *s: _rng.normal(s) * 0.1)(S, Df) * 0.02), 'w_i': _w((lambda *s: _rng.normal(s) * 0.1)(S, Df) * 0.02)}
    _A_in = _A_setup()

    def _B_setup():
        B, S, D, F = (1, 2048, 512, 1376)
        Fh = F // 2
        return {'x': _w((lambda *s: _rng.normal(s) * 0.05)(B, S, D)), 'w_in': _w((lambda *s: _rng.normal(s) * 0.4)(D, 2 * Fh)), 'w_sp': _w(0.01 * (lambda *s: _rng.normal(s) * 0.4)(S, S)), 'b_sp': _w(1.0 + 0.01 * (lambda *s: _rng.normal(s) * 0.05)(S)), 'w_out': _w((lambda *s: _rng.normal(s) * 0.05)(Fh, D))}
    _B_in = _B_setup()
    return {'A_x': _A_in['x'], 'A_w_r': _A_in['w_r'], 'A_w_i': _A_in['w_i'], 'B_x': _B_in['x'], 'B_w_in': _B_in['w_in'], 'B_w_sp': _B_in['w_sp'], 'B_b_sp': _B_in['b_sp'], 'B_w_out': _B_in['w_out']}

def reference(A_x, A_w_r, A_w_i, B_x, B_w_in, B_w_sp, B_b_sp, B_w_out):

    def _A_ref(x, w_r, w_i):
        B, S, D = x.shape
        X = (lambda x, axes=(-2, -1): jnp.fft.rfft2(x.astype(jnp.float32), axes=axes))(x, axes=(-2, -1))
        W = w_r + 1j * w_i
        X = X * W
        y = (lambda x, s, axes=(-2, -1): jnp.fft.irfft2(x, s=s, axes=axes).astype(jnp.bfloat16))(X, (S, D), axes=(-2, -1))
        return y

    def _B_ref(x, w_in, w_sp, b_sp, w_out):
        B, S, D = x.shape
        F = w_in.shape[-1]
        Fh = F // 2
        z = _gelu(jnp.einsum('bsd,df->bsf', x, w_in))
        z1 = z[..., :Fh].copy()
        z2 = _layernorm(z[..., Fh:], axis=-1)
        g = jnp.einsum('ts,bsf->btf', w_sp, z2) + b_sp[None, :, None]
        return jnp.einsum('bsf,fd->bsd', z1 * g, w_out)
    x = A_x
    xn = _layernorm(x, axis=-1)
    s = _A_ref(xn, A_w_r, A_w_i)
    g = _silu(_B_ref(xn, B_w_in, B_w_sp, B_b_sp, B_w_out))
    return x + s * g
```

```python
import functools
import math

import jax
import jax.numpy as jnp
import numpy as np
from jax import lax
import jax.experimental.pallas as pl
import jax.experimental.pallas.tpu as pltpu

S, D, F = 2048, 512, 1376
FH = F // 2
FHP = 768
NS = S // 128
EPS = 1e-5
F32, BF16 = jnp.float32, jnp.bfloat16
_NT = (((1,), (1,)), ((), ()))


@functools.lru_cache(maxsize=1)
def _tables():
    l = np.arange(128)
    kA = 2 * l
    kB = 2 * l + 1
    m0 = (l % 2) == 0
    kAs = kA[(l + 1) % 128]
    n1 = np.arange(128)[:, None].astype(np.float64)

    def cs(k):
        th = 2.0 * np.pi * ((n1 * k[None, :]) % D) / D
        return np.cos(th), np.sin(th)

    cA, sA = cs(kA)
    cAs, sAs = cs(kAs)
    cB, sB = cs(kB)
    F0 = np.where(m0[None, :], cA, -sAs)
    F2 = np.where(m0[None, :], -sAs, cA)
    sg = np.where(kB % 4 == 1, -1.0, 1.0)[None, :]
    F1a, F1b, F1c, F1d = cB, -sB, sg * sB, sg * cB
    cF = np.stack([F0, F2, F1a, F1b, F1c, F1d])

    wA = np.where(kA == 0, 1.0, 2.0)[None, :] / D
    wAs = np.where(kAs == 0, 1.0, 2.0)[None, :] / D
    G0 = np.where(m0[None, :], cA * wA, -sAs * wAs).T
    G2 = np.where(m0[None, :], -sAs * wAs, cA * wA).T
    w2 = 2.0 / D
    G1a, G1b = (cB * w2).T, (-sg * sB * w2).T
    G1c, G1d = (-sB * w2).T, (-sg * cB * w2).T
    cG = np.stack([G0, G2, G1a, G1b, G1c, G1d])

    n2 = np.arange(64)[None, :]
    kh = np.arange(64)[:, None]
    Mf = np.zeros((32, 128, 128))
    for klo in range(32):
        ph = 2.0 * np.pi * ((n2 * (32 * kh + klo)) % S) / S
        c, s = np.cos(ph), np.sin(ph)
        Mf[klo] = np.block([[c, s], [-s, c]])
    Mi = np.transpose(Mf, (0, 2, 1)) / S
    cM = np.stack([Mf, Mi])

    a16 = np.arange(16)
    th16 = 2.0 * np.pi * ((a16[:, None] * a16[None, :]) % 16) / 16
    D16f = np.zeros((128, 128))
    D16f[0:16, :16] = np.cos(th16)
    D16f[16:32, :16] = -np.sin(th16)
    a128 = np.arange(128)
    th128 = 2.0 * np.pi * ((a128[:, None] * a128[None, :]) % 128) / 128
    cS = np.stack([D16f, D16f / (S * D), np.cos(th128), np.sin(th128)])
    tht = 2.0 * np.pi * (a16[:, None] * a128[None, :]) / S
    tw = np.stack([np.cos(tht), np.sin(tht)])

    small = np.concatenate([cF, cG, cS], axis=0)
    return (small.astype(np.float32), cM.astype(np.float32), tw.astype(np.float32))


def _cadd(a, b):
    return (a[0] + b[0], a[1] + b[1])


def _csub(a, b):
    return (a[0] - b[0], a[1] - b[1])


def _dft4(y, sign):
    t0 = _cadd(y[0], y[2])
    t1 = _csub(y[0], y[2])
    t2 = _cadd(y[1], y[3])
    t3 = _csub(y[1], y[3])
    o0 = _cadd(t0, t2)
    o2 = _csub(t0, t2)
    if sign < 0:
        o1 = (t1[0] + t3[1], t1[1] - t3[0])
        o3 = (t1[0] - t3[1], t1[1] + t3[0])
    else:
        o1 = (t1[0] - t3[1], t1[1] + t3[0])
        o3 = (t1[0] + t3[1], t1[1] - t3[0])
    return [o0, o1, o2, o3]


def _ctw(a, num, den, sign):
    num = num % den
    if sign < 0:
        num = (den - num) % den
    if num == 0:
        return a
    if 4 * num == den:
        return (-a[1], a[0])
    if 2 * num == den:
        return (-a[0], -a[1])
    if 4 * num == 3 * den:
        return (a[1], -a[0])
    if (8 * num) % den == 0:
        r = math.sqrt(0.5)
        o = (8 * num) // den
        d = (a[0] - a[1])
        s = (a[0] + a[1])
        if o == 1:
            return (d * r, s * r)
        if o == 3:
            return (s * (-r), d * r)
        if o == 5:
            return (d * (-r), s * (-r))
        return (s * r, d * (-r))
    c = math.cos(2.0 * math.pi * num / den)
    s = math.sin(2.0 * math.pi * num / den)
    return (a[0] * c - a[1] * s, a[0] * s + a[1] * c)


def _dft8(x, sign):
    u = [_cadd(x[k], x[k + 4]) for k in range(4)]
    v = [_csub(x[k], x[k + 4]) for k in range(4)]
    ev = _dft4(u, sign)
    v1 = _ctw(v[1], 1, 8, sign)
    v3 = _ctw(v[3], 3, 8, sign)
    if sign < 0:
        t0 = (v[0][0] + v[2][1], v[0][1] - v[2][0])
        t1 = (v[0][0] - v[2][1], v[0][1] + v[2][0])
    else:
        t0 = (v[0][0] - v[2][1], v[0][1] + v[2][0])
        t1 = (v[0][0] + v[2][1], v[0][1] - v[2][0])
    t2 = _cadd(v1, v3)
    t3 = _csub(v1, v3)
    o1 = _cadd(t0, t2)
    o5 = _csub(t0, t2)
    if sign < 0:
        o3 = (t1[0] + t3[1], t1[1] - t3[0])
        o7 = (t1[0] - t3[1], t1[1] + t3[0])
    else:
        o3 = (t1[0] - t3[1], t1[1] + t3[0])
        o7 = (t1[0] + t3[1], t1[1] - t3[0])
    return [ev[0], o1, ev[1], o3, ev[2], o5, ev[3], o7]


_GC = math.sqrt(2.0 / math.pi)


def _gelu(x):
    inner = x * (x * x * (0.044715 * _GC) + _GC)
    hx = 0.5 * x
    return hx * jnp.tanh(inner) + hx


def _silu(x):
    hx = 0.5 * x
    return hx * jnp.tanh(hx) + hx


def _dot(a, b):
    return jnp.dot(a, b, preferred_element_type=F32)


def _dot_nt(a, b):
    return lax.dot_general(a, b, _NT, preferred_element_type=F32)


def _rows(i, n):
    if isinstance(i, int):
        return pl.ds(i * n, n)
    return pl.ds(pl.multiple_of(i * n, n), n)


def _kernel(x_hbm, wr_hbm, wi_hbm, win_hbm, wsp_hbm, bsp_ref, wout_hbm,
            csm_hbm, cm_hbm, ctw_hbm,
            out_hbm,
            xbuf, wint, csm, cmat, ctw, wbuf, wtr, wsp, wout,
            z2n_ref, z1_ref, y1_ref, p1_ref, v_ref, zz_ref, xm_ref, um_ref,
            gate_ref, obuf, bsp32,
            sem_x, sem_w, sem_sp, sem_o):
    lane = lax.broadcasted_iota(jnp.int32, (1, 128), 1)
    m0 = (lane & 1) == 0
    alt = jnp.where(m0, 1.0, -1.0).astype(F32)

    def x_copy(sig):
        return pltpu.make_async_copy(x_hbm.at[0, _rows(sig, 128), :],
                                     xbuf.at[_rows(sig, 128), :], sem_x.at[sig])

    def sp_copy(sig):
        return pltpu.make_async_copy(wsp_hbm.at[_rows(sig, 128), :],
                                     wsp.at[_rows(sig, 128), :], sem_sp.at[sig])

    def o_copy(sig):
        return pltpu.make_async_copy(obuf.at[_rows(sig, 128), :],
                                     out_hbm.at[0, _rows(sig, 128), :], sem_o.at[sig])

    c_win = [pltpu.make_async_copy(
        win_hbm.at[pl.ds((1 - h) * FH, FH), kd * 128:(kd + 1) * 128],
        wint.at[kd, pl.ds((1 - h) * FH, FH), :], sem_w.at[4 * h + kd])
        for h in range(2) for kd in range(4)]
    c_csm = pltpu.make_async_copy(csm_hbm, csm, sem_w.at[8])
    c_cm = pltpu.make_async_copy(cm_hbm, cmat, sem_w.at[9])
    c_tw = pltpu.make_async_copy(ctw_hbm, ctw, sem_w.at[10])
    c_wout = pltpu.make_async_copy(wout_hbm, wout.at[0:FH, :], sem_w.at[11])
    c_w = [pltpu.make_async_copy(w_hbm, wbuf.at[a], sem_w.at[12 + a])
           for a, w_hbm in enumerate((wr_hbm, wi_hbm))]

    for b in range(4):
        x_copy(4 * b).start()
    for c in c_win[:4]:
        c.start()
    c_csm.start()
    for c in c_win[4:]:
        c.start()
    for j in range(1, 4):
        for b in range(4):
            x_copy(j + 4 * b).start()

    xm_ref[...] = jnp.zeros((128, 128), F32)
    bsp32[...] = bsp_ref[...].astype(F32)
    wout[FH:FHP, :] = jnp.zeros((FHP - FH, D), BF16)

    for c in c_win:
        c.wait()
    c_csm.wait()

    for sig in range(4):
        sp_copy(sig).start()
    for c in c_w:
        c.start()
    c_cm.start()
    c_tw.start()
    c_wout.start()
    for sig in range(4, NS):
        sp_copy(sig).start()

    def wint_rows(r0, n):
        return jnp.concatenate([wint[kd, pl.ds(r0, n), :] for kd in range(4)], axis=1)

    def phase1(j, carry):
        a0s, a2s, pqs = [], [], []
        for b in range(4):
            sig = j + 4 * b
            x_copy(sig).wait()
            xnb, a0c, a2c, pqc = [], [], [], []
            for rc in range(4):
                if isinstance(sig, int):
                    r = pl.ds(sig * 128 + rc * 32, 32)
                else:
                    r = pl.ds(pl.multiple_of(sig * 128 + rc * 32, 32), 32)
                xs = xbuf[r, :].astype(F32)
                mu = jnp.sum(xs, axis=1, keepdims=True) * (1.0 / D)
                xc = xs - mu
                var = jnp.sum(xc * xc, axis=1, keepdims=True) * (1.0 / D)
                xn = xc * lax.rsqrt(var + EPS)
                xnb.append(xn.astype(BF16))
                x0, x1, x2, x3 = [xn[:, t * 128:(t + 1) * 128] for t in range(4)]
                s02 = x0 + x2
                s13 = x1 + x3
                a0 = s02 + s13
                a0c.append(a0.astype(BF16))
                a2c.append((s02 - s13).astype(BF16))
                pqc.append(jnp.concatenate([x0 - x2, x1 - x3], axis=1).astype(BF16))
                nyq = jnp.sum(a0 * alt, axis=1, keepdims=True)
                xm_ref[rc * 32:(rc + 1) * 32, :] = jnp.where(
                    lane == sig, nyq, xm_ref[rc * 32:(rc + 1) * 32, :])
            xnb = jnp.concatenate(xnb, axis=0)
            a0s.append(jnp.concatenate(a0c, axis=0))
            a2s.append(jnp.concatenate(a2c, axis=0))
            pqs.append(jnp.concatenate(pqc, axis=0))

            z2 = _gelu(_dot_nt(wint_rows(FH, FH), xnb))
            m2 = jnp.sum(z2, axis=0, keepdims=True) * (1.0 / FH)
            zc = z2 - m2
            v2 = jnp.sum(zc * zc, axis=0, keepdims=True) * (1.0 / FH)
            z2n_ref[sig] = (zc * lax.rsqrt(v2 + EPS)).astype(BF16)
            z1_ref[sig] = _gelu(_dot_nt(wint_rows(0, FH), xnb))

        t0 = _dot(jnp.concatenate(a0s, axis=0), csm[0])
        t2 = _dot(jnp.concatenate(a2s, axis=0), csm[1])
        f1 = jnp.concatenate([jnp.concatenate([csm[2], csm[3]], axis=1),
                              jnp.concatenate([csm[4], csm[5]], axis=1)], axis=0)
        bb = _dot(jnp.concatenate(pqs, axis=0), f1)
        for rc in range(16):
            ga, gb = [], []
            for b in range(4):
                r0 = b * 128 + rc * 8
                t0c = t0[r0:r0 + 8]
                t2c = t2[r0:r0 + 8]
                re = jnp.where(m0, t0c, t2c)
                im = pltpu.roll(jnp.where(m0, t2c, t0c), 1, 1)
                ga.append((re, im))
                gb.append((bb[r0:r0 + 8, 0:128], bb[r0:r0 + 8, 128:256]))
            if isinstance(j, int):
                r = pl.ds(j * 128 + rc * 8, 8)
            else:
                r = pl.ds(pl.multiple_of(j * 128 + rc * 8, 8), 8)
            for c, g in enumerate((ga, gb)):
                o = _dft4(g, -1)
                for e in range(4):
                    y1_ref[c, 0, e, r, :] = o[e][0]
                    y1_ref[c, 1, e, r, :] = o[e][1]
        return carry

    lax.fori_loop(0, 4, phase1, 0)

    def gate_slab(sig):
        sp_copy(sig).wait()
        z2all = jnp.concatenate([z2n_ref[k] for k in range(NS)], axis=1)
        gt = _dot_nt(z2all, wsp[_rows(sig, 128), :])
        bias = bsp32[pl.ds(sig, 1), :]
        ht = (z1_ref[sig] * (gt + bias)).astype(BF16)
        ht = jnp.concatenate([ht, jnp.zeros((FHP - FH, 128), BF16)], axis=0)
        bo = _dot(ht.T, wout[...])
        return _silu(bo)

    def fft_fwd_radix8():
        for c in range(2):
            for rc in range(4):
                for e in range(4):
                    xs = []
                    for a in range(8):
                        r = pl.ds(a * 64 + rc * 16, 16)
                        xs.append(_ctw((y1_ref[c, 0, e, r, :], y1_ref[c, 1, e, r, :]),
                                       a * e, 32, -1))
                    o = _dft8(xs, -1)
                    for cc in range(8):
                        klo = e + 4 * cc
                        p1_ref[c, klo, pl.ds(rc * 16, 16), :] = o[cc][0].astype(BF16)
                        p1_ref[c, klo, pl.ds(64 + rc * 16, 16), :] = o[cc][1].astype(BF16)

    def w_prep():
        for a in range(2):
            for kb in range(NS):
                wv = pltpu.bitcast(wbuf[a, 0:256, kb * 128:(kb + 1) * 128], jnp.uint32)
                wtr[a, kb * 128:(kb + 1) * 128, :] = wv.T

    def fft_mid():
        for klo in range(32):
            wru = wtr[0, pl.ds(klo, 64, stride=32), :]
            wiu = wtr[1, pl.ds(klo, 64, stride=32), :]
            for c in range(2):
                if c == 0:
                    wr = pltpu.bitcast(wru << 16, F32)
                    wi = pltpu.bitcast(wiu << 16, F32)
                else:
                    wr = pltpu.bitcast(wru & jnp.uint32(0xFFFF0000), F32)
                    wi = pltpu.bitcast(wiu & jnp.uint32(0xFFFF0000), F32)
                xh = _dot(cmat[0, klo], p1_ref[c, klo])
                xr, xi = xh[0:64], xh[64:128]
                yr = xr * wr - xi * wi
                yi = xr * wi + xi * wr
                y = jnp.concatenate([yr.astype(BF16), yi.astype(BF16)], axis=0)
                v_ref[c, klo] = _dot(cmat[1, klo], y)

    def fft_inv_radix8():
        for c in range(2):
            for rc in range(8):
                for e in range(4):
                    xs = []
                    for cc in range(8):
                        klo = e + 4 * cc
                        xs.append((v_ref[c, klo, pl.ds(rc * 8, 8), :],
                                   v_ref[c, klo, pl.ds(64 + rc * 8, 8), :]))
                    o = _dft8(xs, +1)
                    for a in range(8):
                        t = _ctw(o[a], a * e, 32, +1)
                        r = pl.ds(a * 64 + rc * 8, 8)
                        zz_ref[c, 0, e, r, :] = t[0]
                        zz_ref[c, 1, e, r, :] = t[1]

    def nyquist():
        l16 = lax.broadcasted_iota(jnp.int32, (16, 128), 1)
        r16 = lax.broadcasted_iota(jnp.int32, (16, 128), 0)
        idx = 16 * (l16 & 7) + r16
        grp = l16 >> 3
        wn = []
        for a in range(2):
            wrow = wbuf[a, 256:257, :].astype(F32)
            acc = jnp.zeros((16, 128), F32)
            for ka in range(16):
                rowb = jnp.broadcast_to(wrow[:, ka * 128:(ka + 1) * 128], (16, 128))
                acc = jnp.where(grp == ka, jnp.take_along_axis(rowb, idx, axis=1), acc)
            wn.append(acc)
        twc, tws = ctw[0], ctw[1]
        cs128 = jnp.concatenate([csm[14], csm[15]], axis=1)
        aa = _dot_nt(csm[12, 0:32, :], xm_ref[...].astype(BF16))
        ar, ai = aa[0:16], aa[16:32]
        br = ar * twc + ai * tws
        bi = ai * twc - ar * tws
        p = _dot(jnp.concatenate([br, bi], axis=0).astype(BF16), cs128)
        xr = p[0:16, 0:128] + p[16:32, 128:256]
        xi = p[16:32, 0:128] - p[0:16, 128:256]
        yr = xr * wn[0] - xi * wn[1]
        yi = xr * wn[1] + xi * wn[0]
        p = _dot(jnp.concatenate([yr, yi], axis=0).astype(BF16), cs128)
        vr = p[0:16, 0:128] - p[16:32, 128:256]
        vi = p[16:32, 0:128] + p[0:16, 128:256]
        ur = vr * twc - vi * tws
        ui = vi * twc + vr * tws
        u2 = jnp.concatenate([ur, ui, jnp.zeros((96, 128), F32)], axis=0)
        um_ref[...] = _dot(u2.T.astype(BF16), csm[13])

    c_wout.wait()
    gate_ref[0] = gate_slab(0)
    fft_fwd_radix8()
    for c in c_w:
        c.wait()
    w_prep()
    gate_ref[1] = gate_slab(1)
    c_cm.wait()
    c_tw.wait()
    fft_mid()
    nyquist()
    gate_ref[2] = gate_slab(2)
    fft_inv_radix8()
    gate_ref[3] = gate_slab(3)

    def phase3(j, carry):
        gates = [gate_ref[j]] + [gate_slab(j + 4 * b) for b in range(1, 4)]
        t0s = [[] for _ in range(4)]
        t2s = [[] for _ in range(4)]
        ubs = [[] for _ in range(4)]
        for rc in range(8):
            if isinstance(j, int):
                r = pl.ds(j * 128 + rc * 16, 16)
            else:
                r = pl.ds(pl.multiple_of(j * 128 + rc * 16, 16), 16)
            ua = _dft4([(zz_ref[0, 0, e, r, :], zz_ref[0, 1, e, r, :]) for e in range(4)], +1)
            ub = _dft4([(zz_ref[1, 0, e, r, :], zz_ref[1, 1, e, r, :]) for e in range(4)], +1)
            for b in range(4):
                re, im = ua[b]
                ip = pltpu.roll(im, 127, 1)
                t0s[b].append(jnp.where(m0, re, ip).astype(BF16))
                t2s[b].append(jnp.where(m0, ip, re).astype(BF16))
                ubs[b].append(jnp.concatenate([ub[b][0], ub[b][1]], axis=1).astype(BF16))
        cat = lambda parts: jnp.concatenate([p for pb in parts for p in pb], axis=0)
        b0 = _dot(cat(t0s), csm[6])
        b2 = _dot(cat(t2s), csm[7])
        g1 = jnp.concatenate([jnp.concatenate([csm[8], csm[9]], axis=1),
                              jnp.concatenate([csm[10], csm[11]], axis=1)], axis=0)
        pq = _dot(cat(ubs), g1)
        um = um_ref[...]
        for b in range(4):
            sig = j + 4 * b
            col = jnp.sum(jnp.where(lane == sig, um, 0.0), axis=1, keepdims=True)
            for rc in range(8):
                r0 = b * 128 + rc * 16
                b0c = b0[r0:r0 + 16] + col[rc * 16:(rc + 1) * 16] * alt
                b2c = b2[r0:r0 + 16]
                pc = pq[r0:r0 + 16, 0:128]
                qc = pq[r0:r0 + 16, 128:256]
                e02 = b0c + b2c
                o02 = b0c - b2c
                sv = jnp.concatenate([e02 + pc, o02 - qc, e02 - pc, o02 + qc], axis=1)
                if isinstance(sig, int):
                    r = pl.ds(sig * 128 + rc * 16, 16)
                else:
                    r = pl.ds(pl.multiple_of(sig * 128 + rc * 16, 16), 16)
                g = gates[b][rc * 16:(rc + 1) * 16]
                obuf[r, :] = (xbuf[r, :].astype(F32) + sv * g).astype(BF16)
            o_copy(sig).start()
        return carry

    lax.fori_loop(0, 4, phase3, 0)
    for sig in range(NS):
        o_copy(sig).wait()


@jax.jit
def pallas_recurrent_scan__spectral_gfnet__mixer_gmlp__prompt_kernel(
    A_x: jax.Array,
    A_w_r: jax.Array,
    A_w_i: jax.Array,
    B_x: jax.Array,
    B_w_in: jax.Array,
    B_w_sp: jax.Array,
    B_b_sp: jax.Array,
    B_w_out: jax.Array,
):
    del B_x
    small, cm, tw = _tables()
    csm = jnp.asarray(small, dtype=BF16)
    cmat = jnp.asarray(cm, dtype=BF16)
    ctw = jnp.asarray(tw, dtype=F32)
    any_spec = pl.BlockSpec(memory_space=pltpu.HBM)
    scratch = [
        pltpu.VMEM((S, D), BF16),
        pltpu.VMEM((4, F, 128), BF16),
        pltpu.VMEM((16, 128, 128), BF16),
        pltpu.VMEM((2, 32, 128, 128), BF16),
        pltpu.VMEM((2, 16, 128), F32),
        pltpu.VMEM((2, D // 2 + 1, S), BF16),
        pltpu.VMEM((2, S, 128), jnp.uint32),
        pltpu.VMEM((S, S), BF16),
        pltpu.VMEM((FHP, D), BF16),
        pltpu.VMEM((NS, FH, 128), BF16),
        pltpu.VMEM((NS, FH, 128), F32),
        pltpu.VMEM((2, 2, 4, 512, 128), F32),
        pltpu.VMEM((2, 32, 128, 128), BF16),
        pltpu.VMEM((2, 32, 128, 128), F32),
        pltpu.VMEM((2, 2, 4, 512, 128), F32),
        pltpu.VMEM((128, 128), F32),
        pltpu.VMEM((128, 128), F32),
        pltpu.VMEM((4, 128, D), F32),
        pltpu.VMEM((S, D), BF16),
        pltpu.VMEM((NS, 128), F32),
        pltpu.SemaphoreType.DMA((NS,)),
        pltpu.SemaphoreType.DMA((14,)),
        pltpu.SemaphoreType.DMA((NS,)),
        pltpu.SemaphoreType.DMA((NS,)),
    ]
    return pl.pallas_call(
        _kernel,
        out_shape=jax.ShapeDtypeStruct((1, S, D), BF16),
        in_specs=[any_spec, any_spec, any_spec, any_spec, any_spec,
                  pl.BlockSpec(memory_space=pltpu.VMEM), any_spec,
                  any_spec, any_spec, any_spec],
        out_specs=any_spec,
        scratch_shapes=scratch,
        compiler_params=pltpu.CompilerParams(vmem_limit_bytes=100 * 1024 * 1024),
    )(A_x, A_w_r.T, A_w_i.T, B_w_in.T, B_w_sp, B_b_sp.reshape(NS, 128), B_w_out,
      csm, cmat, ctw)
```

```python
import functools
import math

import jax
import jax.numpy as jnp
import numpy as np
from jax import lax
import jax.experimental.pallas as pl
import jax.experimental.pallas.tpu as pltpu

S, D, F = 2048, 512, 1376
FH = F // 2
FHP = 768
NS = S // 128
EPS = 1e-5
F32, BF16, U32 = jnp.float32, jnp.bfloat16, jnp.uint32
WP = 33
_NT = (((1,), (1,)), ((), ()))
_C1 = math.sqrt(2.0 / math.pi)
ALPHA = (0.044715 * _C1) ** (1.0 / 3.0)
GC = _C1 / ALPHA


@functools.lru_cache(maxsize=1)
def _tables():
    l = np.arange(128)
    kA = 2 * l
    kB = 2 * l + 1
    m0 = (l % 2) == 0
    kAs = kA[(l + 1) % 128]
    n1 = np.arange(128)[:, None].astype(np.float64)

    def cs(k):
        th = 2.0 * np.pi * ((n1 * k[None, :]) % D) / D
        return np.cos(th), np.sin(th)

    cA, sA = cs(kA)
    cAs, sAs = cs(kAs)
    cB, sB = cs(kB)
    F0 = np.where(m0[None, :], cA, -sAs)
    F2 = np.where(m0[None, :], -sAs, cA)
    sg = np.where(kB % 4 == 1, -1.0, 1.0)[None, :]
    F1a, F1b, F1c, F1d = cB, -sB, sg * sB, sg * cB
    cF = np.stack([F0, F2, F1a, F1b, F1c, F1d]) / ALPHA

    wA = np.where(kA == 0, 1.0, 2.0)[None, :] / D
    wAs = np.where(kAs == 0, 1.0, 2.0)[None, :] / D
    G0 = np.where(m0[None, :], cA * wA, -sAs * wAs).T
    G0[127, :] = np.where(m0, 1.0, -1.0) / D
    G2 = np.where(m0[None, :], -sAs * wAs, cA * wA).T
    w2 = 2.0 / D
    G1a, G1b = (cB * w2).T, (-sg * sB * w2).T
    G1c, G1d = (-sB * w2).T, (-sg * cB * w2).T
    cG = np.stack([G0, G2, G1a, G1b, G1c, G1d])

    n2 = np.arange(64)[None, :]
    kh = np.arange(64)[:, None]
    Mf = np.zeros((32, 128, 128))
    for klo in range(32):
        ph = 2.0 * np.pi * ((n2 * (32 * kh + klo)) % S) / S
        c, s = np.cos(ph), np.sin(ph)
        Mf[klo] = np.block([[c, s], [-s, c]])
    Mi = np.transpose(Mf, (0, 2, 1)) / S
    cM = np.stack([Mf, Mi])

    a16 = np.arange(16)
    th16 = 2.0 * np.pi * ((a16[:, None] * a16[None, :]) % 16) / 16
    D16f = np.zeros((128, 128))
    D16f[0:16, :16] = np.cos(th16)
    D16f[16:32, :16] = -np.sin(th16)
    a128 = np.arange(128)
    th128 = 2.0 * np.pi * ((a128[:, None] * a128[None, :]) % 128) / 128
    cS = np.stack([D16f / ALPHA, D16f / S, np.cos(th128), np.sin(th128)])
    tht = 2.0 * np.pi * (a16[:, None] * a128[None, :]) / S
    tw = np.stack([np.cos(tht), np.sin(tht)])

    small = np.concatenate([cF, cG, cS], axis=0)
    return (small.astype(np.float32), cM.astype(np.float32), tw.astype(np.float32))


def _cadd(a, b):
    return (a[0] + b[0], a[1] + b[1])


def _csub(a, b):
    return (a[0] - b[0], a[1] - b[1])


def _dft4(y, sign):
    t0 = _cadd(y[0], y[2])
    t1 = _csub(y[0], y[2])
    t2 = _cadd(y[1], y[3])
    t3 = _csub(y[1], y[3])
    o0 = _cadd(t0, t2)
    o2 = _csub(t0, t2)
    if sign < 0:
        o1 = (t1[0] + t3[1], t1[1] - t3[0])
        o3 = (t1[0] - t3[1], t1[1] + t3[0])
    else:
        o1 = (t1[0] - t3[1], t1[1] + t3[0])
        o3 = (t1[0] + t3[1], t1[1] - t3[0])
    return [o0, o1, o2, o3]


def _ctw(a, num, den, sign):
    num = num % den
    if sign < 0:
        num = (den - num) % den
    if num == 0:
        return a
    if 4 * num == den:
        return (-a[1], a[0])
    if 2 * num == den:
        return (-a[0], -a[1])
    if 4 * num == 3 * den:
        return (a[1], -a[0])
    if (8 * num) % den == 0:
        r = math.sqrt(0.5)
        o = (8 * num) // den
        d = (a[0] - a[1])
        s = (a[0] + a[1])
        if o == 1:
            return (d * r, s * r)
        if o == 3:
            return (s * (-r), d * r)
        if o == 5:
            return (d * (-r), s * (-r))
        return (s * r, d * (-r))
    c = math.cos(2.0 * math.pi * num / den)
    s = math.sin(2.0 * math.pi * num / den)
    return (a[0] * c - a[1] * s, a[0] * s + a[1] * c)


def _dft8(x, sign):
    u = [_cadd(x[k], x[k + 4]) for k in range(4)]
    v = [_csub(x[k], x[k + 4]) for k in range(4)]
    ev = _dft4(u, sign)
    v1 = _ctw(v[1], 1, 8, sign)
    v3 = _ctw(v[3], 3, 8, sign)
    if sign < 0:
        t0 = (v[0][0] + v[2][1], v[0][1] - v[2][0])
        t1 = (v[0][0] - v[2][1], v[0][1] + v[2][0])
    else:
        t0 = (v[0][0] - v[2][1], v[0][1] + v[2][0])
        t1 = (v[0][0] + v[2][1], v[0][1] - v[2][0])
    t2 = _cadd(v1, v3)
    t3 = _csub(v1, v3)
    o1 = _cadd(t0, t2)
    o5 = _csub(t0, t2)
    if sign < 0:
        o3 = (t1[0] + t3[1], t1[1] - t3[0])
        o7 = (t1[0] - t3[1], t1[1] + t3[0])
    else:
        o3 = (t1[0] - t3[1], t1[1] + t3[0])
        o7 = (t1[0] + t3[1], t1[1] - t3[0])
    return [ev[0], o1, ev[1], o3, ev[2], o5, ev[3], o7]


def _gelu2a(xs):
    return xs * jnp.tanh(xs * (xs * xs + GC)) + xs


def _silu_h(hx):
    return hx * jnp.tanh(hx) + hx


def _dot(a, b):
    return jnp.dot(a, b, preferred_element_type=F32)


def _dot_nt(a, b):
    return lax.dot_general(a, b, _NT, preferred_element_type=F32)


def _rows(i, n):
    if isinstance(i, int):
        return pl.ds(i * n, n)
    return pl.ds(pl.multiple_of(i * n, n), n)


def _ds(start, n):
    if isinstance(start, int):
        return pl.ds(start, n)
    return pl.ds(pl.multiple_of(start, n), n)


def _kernel(x_hbm, wr_hbm, wi_hbm, win_hbm, wsp_hbm, bsp_hbm, wout_hbm,
            csm_hbm, cm_hbm, ctw_hbm, zero_hbm,
            out_hbm,
            xbuf, wint, csm, cmat, ctw, wbuf, wtr, wsp, wout, bspb, zsm,
            z2n_ref, z1_ref, y1_ref, zz_ref, xm_ref, um_ref,
            gate_ref, tin, sbuf, obuf, bsp32,
            sem_x, sem_w, sem_sp, sem_o, *bufs):
    p1_refs, v_refs, yb_refs = bufs[0:4], bufs[4:8], bufs[8:12]
    zd_refs, lnb = bufs[12:14], bufs[14:30]
    hb_refs, gcar = bufs[30:32], bufs[32]
    hb_u = [r.bitcast(U32) for r in hb_refs]
    lane = lax.broadcasted_iota(jnp.int32, (1, 128), 1)
    m0 = (lane & 1) == 0
    alt = jnp.where(m0, 1.0, -1.0).astype(F32)

    wint_u, csm_u, cmat_u = wint.bitcast(U32), csm.bitcast(U32), cmat.bitcast(U32)
    z2n_u, wout_u = z2n_ref.bitcast(U32), wout.bitcast(U32)
    lnb_u, tin_u = [r.bitcast(U32) for r in lnb], tin.bitcast(U32)
    yb_u = [r.bitcast(U32) for r in yb_refs]

    def _bf(v):
        return pltpu.bitcast(v, BF16)

    def cs(i):
        return _bf(csm_u[i])

    def x_copy(sig):
        return pltpu.make_async_copy(x_hbm.at[0, _rows(sig, 128), :],
                                     xbuf.at[_rows(sig, 128), :], sem_x.at[sig])

    def sp_copy(sig):
        return pltpu.make_async_copy(wsp_hbm.at[_rows(sig, 128), :],
                                     wsp.at[_rows(sig, 128), :], sem_sp.at[sig])

    def o_copy(sig):
        return pltpu.make_async_copy(obuf.at[_rows(sig, 128), :],
                                     out_hbm.at[0, _rows(sig, 128), :], sem_o.at[sig])

    c_win = [pltpu.make_async_copy(
        win_hbm.at[pl.ds((1 - h) * FH, FH), kd * 128:(kd + 1) * 128],
        wint.at[kd, pl.ds((1 - h) * FH, FH), :], sem_w.at[4 * h + kd])
        for h in range(2) for kd in range(4)]
    c_csf = pltpu.make_async_copy(csm_hbm.at[0:6], csm.at[0:6], sem_w.at[8])
    c_csr = pltpu.make_async_copy(csm_hbm.at[6:16], csm.at[6:16], sem_w.at[18])
    c_cm = pltpu.make_async_copy(cm_hbm, cmat, sem_w.at[9])
    c_tw = pltpu.make_async_copy(ctw_hbm, ctw, sem_w.at[10])
    c_bsp = pltpu.make_async_copy(bsp_hbm, bspb, sem_w.at[11])
    c_w = [pltpu.make_async_copy(w_hbm, wbuf.at[a], sem_w.at[12 + a])
           for a, w_hbm in enumerate((wr_hbm, wi_hbm))]
    c_wout = [pltpu.make_async_copy(wout_hbm.at[:, nt * 128:(nt + 1) * 128],
                                    wout.at[nt, 0:FH, :], sem_w.at[14 + nt])
              for nt in range(4)]
    c_zero = pltpu.make_async_copy(zero_hbm, zsm, sem_w.at[19])

    x_copy(0).start()
    c_zero.start()
    for c in c_win[:4]:
        c.start()
    x_copy(4).start()

    xm_ref[...] = jnp.zeros((128, 128), F32)
    wout[:, FH:FHP, :] = jnp.zeros((4, FHP - FH, 128), BF16)

    x_copy(0).wait()
    c_zero.wait()
    for c in c_win[4:]:
        c.start()
    for sig in (8, 12, 1, 5):
        x_copy(sig).start()
    c_csf.start()

    zero = zsm[0]
    never = jnp.full((8, 128), zero, jnp.int32) > 0

    pending = []

    def attach(p, vals, lo=0, hi=None):
        n = len(vals)
        if n == 0:
            return p
        nr = p.shape[0] // 8
        hi = nr if hi is None else hi
        at = {lo + ((u + 1) * (hi - lo)) // n - 1: vals[u] for u in range(n)}
        assert len(at) == n
        parts, r0 = [], 0
        for r in sorted(at):
            if r > r0:
                parts.append(p[r0 * 8:r * 8])
            parts.append(jnp.where(never, at[r], p[r * 8:(r + 1) * 8]))
            r0 = r + 1
        if r0 < nr:
            parts.append(p[r0 * 8:])
        return jnp.concatenate(parts, axis=0)

    def fenced(p, units, lo=0):
        return attach(p, [u() for u in units], lo)

    def drain(p, hi=None, lo=8):
        vals = [pltpu.bitcast(v, U32) for v in pending]
        del pending[:]
        return attach(p, vals, lo, hi)

    def ln_unit(sig, rc):
        def run(gate=None):
            xs = xbuf[pl.ds(sig * 128 + rc * 16, 16), :].astype(F32)
            if gate is not None:
                x00 = jnp.concatenate([jnp.where(never, gate, xs[0:8, 0:128]),
                                       jnp.where(never, gate, xs[8:16, 0:128])], axis=0)
                xs = jnp.concatenate([x00, xs[:, 128:]], axis=1)
            mu = jnp.sum(xs, axis=1, keepdims=True) * (1.0 / D)
            xc = xs - mu
            var = jnp.sum(xc * xc, axis=1, keepdims=True) * (1.0 / D)
            xn = xc * (lax.rsqrt(var + EPS) * ALPHA)
            x0, x1, x2, x3 = [xn[:, t * 128:(t + 1) * 128] for t in range(4)]
            s02 = x0 + x2
            s13 = x1 + x3
            a0 = s02 + s13
            r = pl.ds(rc * 16, 16)
            q = x1 - x3
            for t, val in enumerate((x0, x1, x2, x3, a0, s02 - s13, x0 - x2, q)):
                lnb[sig][t, r, :] = val.astype(BF16)
            nyq = jnp.sum(a0 * alt, axis=1, keepdims=True)
            nyq = jnp.broadcast_to(nyq, (16, 128))
            pltpu.store(xm_ref.at[r, :], nyq,
                        mask=jnp.broadcast_to(lane == sig, (16, 128)))
            pending.append(nyq[0:8] + nyq[8:16])
        return run

    def wint_rows(r0, n):
        tiles = [wint_u[kd, pl.ds(r0 // 2, n // 2), :] for kd in range(4)]
        tiles[0] = drain(tiles[0], 30 if r0 == 0 else None)
        return jnp.concatenate([_bf(t) for t in tiles], axis=1)

    def xn_slab(sig):
        return jnp.concatenate([_bf(lnb_u[sig][t + zero]) for t in range(4)], axis=1)

    def z2_part(sig, units):
        zd = zd_refs[sig_slot[sig]]
        p = _dot_nt(wint_rows(FH, FH), xn_slab(sig))
        for u, unit in enumerate(units):
            unit(p[u * 64:u * 64 + 8])
        c0 = s1 = s2 = None
        hist = []
        for i in range(11):
            n = 8 if i < 10 else 6
            v = p[i * 64:i * 64 + 8 * n]
            if i >= 2:
                v = jnp.concatenate([jnp.where(never, hist[i - 2][0], v[0:8]),
                                     jnp.where(never, hist[i - 2][1], v[8:16]),
                                     v[16:]], axis=0)
            y = _gelu2a(v).reshape(n, 8, 128)
            if i == 0:
                c0 = y[0]
            d = y - c0
            zd[i, 0:8 * n, :] = d.reshape(8 * n, 128)
            t1 = jnp.sum(d, axis=0)
            t2 = jnp.sum(d * d, axis=0)
            s1 = t1 if s1 is None else s1 + t1
            s2 = t2 if s2 is None else s2 + t2
            hist.append((s1, s2))
        ng = FH // 8
        mean_g = c0 + s1 * (1.0 / ng)
        mean = jnp.sum(mean_g, axis=0, keepdims=True) * 0.125
        dm = mean_g - mean
        m2 = s2 - s1 * s1 * (1.0 / ng) + dm * dm * float(ng)
        var = jnp.maximum(jnp.sum(m2, axis=0, keepdims=True) * (1.0 / FH), 0.0)
        rs = lax.rsqrt(var + EPS * (4.0 * ALPHA * ALPHA)) * (0.25 / ALPHA)
        rs = jnp.broadcast_to(rs, (8, 128))
        sh = (c0 - mean) * rs

        def norm_unit(i):
            def run(gate):
                n = 8 if i < 10 else 6
                ri = jnp.where(never, gate, rs)
                d = zd[i + zero, 0:8 * n, :].reshape(n, 8, 128)
                z2n_ref[sig, pl.ds(i * 64, 8 * n), :] = (
                    (d * ri + sh).reshape(8 * n, 128).astype(BF16))
            return run
        return [norm_unit(i) for i in range(11)]

    def z1_part(sig, ln_units, norm_units):
        p = _dot_nt(wint_rows(0, FH), xn_slab(sig))
        for u, unit in enumerate(ln_units):
            unit(p[u * 64:u * 64 + 8])
        for u, unit in enumerate(norm_units):
            unit(p[u * 56 + 64:u * 56 + 72])
        z1_ref[sig] = _gelu2a(p)

    def d_fwd(j):
        def lhs(planes, rcs):
            return jnp.concatenate(
                [jnp.concatenate([_bf(lnb_u[j + 4 * b][t + zero, pl.ds(rc * 8, 8), :])
                                  for t in planes], axis=1)
                 for rc in rcs for b in range(4)], axis=0)
        halves = (range(0, 4), range(4, 8))
        t0 = jnp.concatenate([_dot(lhs((4,), h), cs(0)) for h in halves], axis=0)
        t2 = jnp.concatenate([_dot(lhs((5,), h), cs(1)) for h in halves], axis=0)
        f1 = jnp.concatenate([jnp.concatenate([cs(2), cs(3)], axis=1),
                              jnp.concatenate([cs(4), cs(5)], axis=1)], axis=0)
        bb = _dot(lhs((6, 7), range(8)), f1)
        for c in range(2):
            for rc in range(16):
                g = []
                for b in range(4):
                    r0 = (rc // 2) * 64 + b * 16 + (rc % 2) * 8
                    if c == 0:
                        t0c = t0[r0:r0 + 8]
                        t2c = t2[r0:r0 + 8]
                        g.append((jnp.where(m0, t0c, t2c),
                                  pltpu.roll(jnp.where(m0, t2c, t0c), 1, 1)))
                    else:
                        g.append((bb[r0:r0 + 8, 0:128], bb[r0:r0 + 8, 128:256]))
                o = _dft4(g, -1)
                if c == 0:
                    pending.append(o[0][1])
                r = pl.ds(j * 128 + rc * 8, 8)
                for e in range(4):
                    y1_ref[c, 0, e, r, :] = o[e][0]
                    y1_ref[c, 1, e, r, :] = o[e][1]

    for rc in range(8):
        ln_unit(0, rc)()
    for c in c_win[:4]:
        c.wait()
    x_copy(4).wait()
    order = [j + 4 * b for j in range(4) for b in range(4)]
    sig_slot = {sig: idx % 2 for idx, sig in enumerate(order)}
    def lns(idx):
        return [ln_unit(order[idx], rc) for rc in range(8)] if idx < NS else []

    norms0 = z2_part(order[0], lns(1))
    norms1 = z2_part(order[1], [])
    for c in c_win[4:]:
        c.wait()
    for s2 in (8, 12, 1, 5):
        x_copy(s2).wait()
    c_csf.wait()
    for s2 in range(NS):
        if s2 not in (0, 4, 8, 12, 1, 5):
            x_copy(s2).start()
    for s2 in range(4):
        sp_copy(s2).start()
    for c in c_w + [c_cm, c_bsp] + c_wout + [c_tw, c_csr]:
        c.start()
    for s2 in range(4, NS):
        sp_copy(s2).start()
    z1_part(order[0], lns(2), norms0)
    z1_part(order[1], [], norms1)
    for idx in range(2, NS):
        sig = order[idx]
        if idx == 4:
            for s2 in range(NS):
                if s2 not in (0, 4, 8, 12, 1, 5):
                    x_copy(s2).wait()
        norms = z2_part(sig, lns(idx + 1))
        z1_part(sig, [], norms)
        if idx % 4 == 2:
            d_fwd(idx // 4)

    class Gate:
        def __init__(self, sig):
            self.sig = sig
            self.acc = None

        def k(self, g, units=(), lo=0):
            tiles = [z2n_u[4 * g + t] for t in range(4)]
            tiles[0] = drain(tiles[0], 40, 22)
            lhs = jnp.concatenate([_bf(t) for t in tiles], axis=1)
            p = _dot_nt(lhs, wsp[_rows(self.sig, 128), g * 512:(g + 1) * 512])
            self.mid = p[400:408]
            p = fenced(p, list(units), lo)
            self.acc = p if self.acc is None else self.acc + p

    def h_tiles(sig, acc, slot):
        bias = bsp32[pl.ds(sig, 1), :]
        for t in range(6):
            n = 128 if t < 5 else FH - 640
            ht = z1_ref[sig, pl.ds(t * 128, n), :] * (acc[t * 128:t * 128 + n] + bias)
            if n < 128:
                ht = jnp.concatenate([ht, jnp.zeros((128 - n, 128), F32)], axis=0)
            ht = ht.astype(BF16).T
            hb_refs[slot][t] = ht
            pending.append(pltpu.bitcast(ht[112:128], F32))

    def small(slot, after=None):
        tiles = [hb_u[slot][t + zero] for t in range(6)]
        if after is not None:
            tiles[0] = attach(tiles[0], [pltpu.bitcast(after.mid, U32)], 0, 1)
        h = jnp.concatenate([_bf(t) for t in tiles], axis=1)
        wo = jnp.concatenate([_bf(wout_u[nt]) for nt in range(4)], axis=1)
        return _silu_h(_dot(h, wo))

    def save_acc(acc):
        gcar[0] = acc[0:FH // 2]
        gcar[1] = acc[FH // 2:FH]

    def load_acc():
        return jnp.concatenate([gcar[zero], gcar[1 + zero]], axis=0)

    def f_unit(c, e, rc):
        def run():
            xs = []
            for a in range(8):
                r = pl.ds(a * 64 + rc * 8, 8)
                xs.append(_ctw((y1_ref[c + zero, 0, e, r, :], y1_ref[c + zero, 1, e, r, :]),
                               a * e, 32, -1))
            o = _dft8(xs, -1)
            for cc in range(8):
                p1_refs[e][c, cc, pl.ds(rc * 8, 8), :] = o[cc][0]
                p1_refs[e][c, cc, pl.ds(64 + rc * 8, 8), :] = o[cc][1]
            return o[7][1]
        return run

    def f_units(e):
        return [f_unit(c, e, rc) for c in range(2) for rc in range(8)]

    def w_unit(a, kb):
        def run():
            wt = pltpu.bitcast(wbuf[a, 0:256, kb * 128:(kb + 1) * 128], U32).T
            for h in range(4):
                wtr[a, pl.ds((4 * kb + h) * WP, 32), :] = wt[h * 32:(h + 1) * 32]
            return pltpu.bitcast(wt[120:128], F32)
        return run

    def mid1(e):
        for cc in range(8):
            klo = e + 4 * cc
            wru = wtr[0, pl.ds(klo, 64, stride=WP), :]
            wiu = wtr[1, pl.ds(klo, 64, stride=WP), :]
            for c in range(2):
                if c == 0:
                    wr = pltpu.bitcast(wru << 16, F32)
                    wi = pltpu.bitcast(wiu << 16, F32)
                else:
                    wr = pltpu.bitcast(wru & jnp.uint32(0xFFFF0000), F32)
                    wi = pltpu.bitcast(wiu & jnp.uint32(0xFFFF0000), F32)
                xh = _dot(_bf(cmat_u[0, klo]), p1_refs[e][c + zero, cc].astype(BF16))
                xr, xi = xh[0:64], xh[64:128]
                yb_refs[e][c, cc, 0:64, :] = (xr * wr - xi * wi).astype(BF16)
                yb_refs[e][c, cc, 64:128, :] = (xr * wi + xi * wr).astype(BF16)

    def mid2(e):
        for cc in range(8):
            klo = e + 4 * cc
            for c in range(2):
                v_refs[e][c, cc] = _dot(_bf(cmat_u[1, klo]), _bf(yb_u[e][c + zero, cc]))

    def i_unit(c, e, rc):
        def run():
            xs = []
            for cc in range(8):
                xs.append((v_refs[e][c + zero, cc, pl.ds(rc * 8, 8), :],
                           v_refs[e][c + zero, cc, pl.ds(64 + rc * 8, 8), :]))
            o = _dft8(xs, +1)
            for a in range(8):
                t = _ctw(o[a], a * e, 32, +1)
                r = pl.ds(a * 64 + rc * 8, 8)
                zz_ref[c, 0, e, r, :] = t[0]
                zz_ref[c, 1, e, r, :] = t[1]
            return t[1]
        return run

    def i_units(e):
        return [i_unit(c, e, rc) for c in range(2) for rc in range(8)]

    nq = {}

    def nyq0():
        twc, tws = ctw[0], ctw[1]
        aa = _dot_nt(_bf(csm_u[12, 0:16, :]), xm_ref[...].astype(BF16))
        ar, ai = aa[0:16], aa[16:32]
        nq[0] = jnp.concatenate([ar * twc + ai * tws, ai * twc - ar * tws], axis=0)

    def nyq1():
        l16 = lax.broadcasted_iota(jnp.int32, (16, 128), 1)
        r16 = lax.broadcasted_iota(jnp.int32, (16, 128), 0)
        idx = 16 * (l16 & 7) + r16
        grp = l16 >> 3
        wn = []
        for a in range(2):
            wrow = wbuf[a, 256:257, :].astype(F32)
            acc = jnp.zeros((16, 128), F32)
            for ka in range(16):
                rowb = jnp.broadcast_to(wrow[:, ka * 128:(ka + 1) * 128], (16, 128))
                acc = jnp.where(grp == ka, jnp.take_along_axis(rowb, idx, axis=1), acc)
            wn.append(acc)
        cs128 = jnp.concatenate([cs(14), cs(15)], axis=1)
        p = _dot(nq[0].astype(BF16), cs128)
        xr = p[0:16, 0:128] + p[16:32, 128:256]
        xi = p[16:32, 0:128] - p[0:16, 128:256]
        nq[1] = jnp.concatenate([xr * wn[0] - xi * wn[1], xr * wn[1] + xi * wn[0]], axis=0)

    def nyq2():
        twc, tws = ctw[0], ctw[1]
        cs128 = jnp.concatenate([cs(14), cs(15)], axis=1)
        p = _dot(nq[1].astype(BF16), cs128)
        vr = p[0:16, 0:128] - p[16:32, 128:256]
        vi = p[16:32, 0:128] + p[0:16, 128:256]
        nq[2] = jnp.concatenate([vr * twc - vi * tws, vi * twc + vr * tws,
                                 jnp.zeros((96, 128), F32)], axis=0)

    def nyq3():
        um_ref[...] = _dot(nq[2].T.astype(BF16), cs(13))

    for c in (c_wout + c_w + [c_cm, c_tw, c_bsp, c_csr]
              + [sp_copy(sig) for sig in range(4)]):
        c.wait()
    bsp32[...] = bspb[...].astype(F32) * (0.25 / ALPHA)
    wu = [w_unit(a, kb) for kb in range(NS) for a in range(2)]
    g0, g1, g2, g3 = Gate(0), Gate(1), Gate(2), Gate(3)
    f1 = f_units(1)
    i3 = i_units(3)
    g0.k(0, f_units(0))
    g0.k(1, wu[:16])
    g0.k(2, wu[16:])
    nyq0()
    g0.k(3, f1[:8])
    mid1(0)
    h_tiles(0, g0.acc, 0)
    g1.k(0, f1[8:], 20)
    gate_ref[0] = small(0, g1)
    mid2(0)
    nyq1()
    g1.k(1, i_units(0))
    mid1(1)
    g1.k(2, f_units(2), 20)
    mid2(1)
    nyq2()
    g1.k(3, i_units(1))
    mid1(2)
    h_tiles(1, g1.acc, 1)
    g2.k(0, f_units(3), 20)
    gate_ref[1] = small(1, g2)
    mid2(2)
    nyq3()
    g2.k(1, i_units(2))
    mid1(3)
    g2.k(2)
    mid2(3)
    g2.k(3, i3[:8])
    h_tiles(2, g2.acc, 0)
    g3.k(0, i3[8:])
    gate_ref[2] = small(0, g3)
    g3.k(1)
    g3.k(2)
    g3.k(3)
    save_acc(g3.acc)
    sbuf[2] = jnp.zeros((128, D), F32)

    def emit(sig, rc, sv, g, dst=None):
        r = _ds(sig * 128 + rc * 16, 16)
        ro = r if dst is None else _ds(dst * 128 + rc * 16, 16)
        obuf[ro, :] = (xbuf[r, :].astype(F32) + sv * g).astype(BF16)

    def finish(sig, b, g, dst=None):
        for rc in range(8):
            emit(sig, rc, sbuf[b - 1 + zero, pl.ds(rc * 16, 16), :],
                 g[rc * 16:(rc + 1) * 16], dst)

    def phase3(j, carry):
        for b in range(1, 4):
            sp_copy(j + 4 * b).wait()

        def r_unit(c, rc):
            def run():
                r = _ds(j * 128 + rc * 16, 16)
                u = _dft4([(zz_ref[c, 0, e, r, :], zz_ref[c, 1, e, r, :])
                           for e in range(4)], +1)
                for b in range(4):
                    ro = pl.ds(rc * 64 + b * 16, 16)
                    re, im = u[b]
                    if c == 0:
                        nq_col = pltpu.roll(um_ref[pl.ds(rc * 16, 16), :],
                                            (128 - 4 * b - j) % 128, 1)
                        ip = pltpu.roll(jnp.where(lane == 0, nq_col, im), 127, 1)
                        tin[0, ro, :] = jnp.where(m0, re, ip).astype(BF16)
                        tin[1, ro, :] = jnp.where(m0, ip, re).astype(BF16)
                    else:
                        tin[2, ro, :] = re.astype(BF16)
                        tin[3, ro, :] = im.astype(BF16)
                return ip[8:16] if c == 0 else u[3][1][8:16]
            return run

        def d_inv():
            hv = (pl.ds(0, 128), pl.ds(128, 128))
            b0 = jnp.concatenate([_dot(_bf(tin_u[zero, h, :]), cs(6)) for h in hv], axis=0)
            b2 = jnp.concatenate([_dot(_bf(tin_u[1 + zero, h, :]), cs(7)) for h in hv], axis=0)
            g1m = jnp.concatenate([jnp.concatenate([cs(8), cs(9)], axis=1),
                                   jnp.concatenate([cs(10), cs(11)], axis=1)], axis=0)
            pq = _dot(jnp.concatenate([_bf(tin_u[2 + zero]), _bf(tin_u[3 + zero])], axis=1),
                      g1m)
            for rc in range(8):
                for b in range(4):
                    r0 = rc * 64 + b * 16
                    b0c = b0[r0:r0 + 16]
                    b2c = b2[r0:r0 + 16]
                    pc = pq[r0:r0 + 16, 0:128]
                    qc = pq[r0:r0 + 16, 128:256]
                    e02 = b0c + b2c
                    o02 = b0c - b2c
                    sv = jnp.concatenate([e02 + pc, o02 - qc, e02 - pc, o02 + qc], axis=1)
                    if b == 0:
                        emit(j, rc, sv, gate_ref[j, pl.ds(rc * 16, 16), :])
                    else:
                        sbuf[b - 1, pl.ds(rc * 16, 16), :] = sv

        first = j == 0
        car = jnp.where(first, 3, j + 11)
        ga, gb, gc = Gate(j + 4), Gate(j + 8), Gate(j + 12)
        h_tiles(car, load_acc(), 1)
        ga.k(0, [r_unit(c, rc) for rc in range(8) for c in range(2)])
        g = small(1, ga)
        gate_ref[jnp.where(first, 3, 4)] = g
        finish(car, 3, g, jnp.where(first, NS, car))
        ga.k(1)
        d_inv()
        ga.k(2)
        ga.k(3)
        h_tiles(j + 4, ga.acc, 0)
        gb.k(0)
        finish(j + 4, 1, small(0, gb))
        gb.k(1)
        gb.k(2)
        gb.k(3)
        h_tiles(j + 8, gb.acc, 1)
        gc.k(0)
        finish(j + 8, 2, small(1, gc))
        gc.k(1)
        gc.k(2)
        gc.k(3)
        save_acc(gc.acc)
        for b in range(3):
            o_copy(j + 4 * b).start()

        @pl.when(j > 0)
        def _():
            o_copy(j + 11).start()
        return carry

    lax.fori_loop(0, 4, phase3, 0)
    h_tiles(NS - 1, load_acc(), 1)
    del pending[:]
    finish(NS - 1, 3, small(1))
    o_copy(NS - 1).start()
    for sig in range(NS):
        o_copy(sig).wait()


@jax.jit
def pallas_recurrent_scan__spectral_gfnet__mixer_gmlp__prompt_kernel(
    A_x: jax.Array,
    A_w_r: jax.Array,
    A_w_i: jax.Array,
    B_x: jax.Array,
    B_w_in: jax.Array,
    B_w_sp: jax.Array,
    B_b_sp: jax.Array,
    B_w_out: jax.Array,
):
    del B_x
    small, cm, tw = _tables()
    csm = jnp.asarray(small, dtype=BF16)
    cmat = jnp.asarray(cm, dtype=BF16)
    ctw = jnp.asarray(tw, dtype=F32)
    zero = jnp.zeros((1,), jnp.int32)
    hbm = pl.BlockSpec(memory_space=pltpu.HBM)
    scratch = [
        pltpu.VMEM((S, D), BF16),
        pltpu.VMEM((4, F, 128), BF16),
        pltpu.VMEM((16, 128, 128), BF16),
        pltpu.VMEM((2, 32, 128, 128), BF16),
        pltpu.VMEM((2, 16, 128), F32),
        pltpu.VMEM((2, D // 2 + 1, S), BF16),
        pltpu.VMEM((2, 64 * WP, 128), U32),
        pltpu.VMEM((S, S), BF16),
        pltpu.VMEM((4, FHP, 128), BF16),
        pltpu.VMEM((NS, 128), BF16),
        pltpu.SMEM((1,), jnp.int32),
        pltpu.VMEM((NS, FH, 128), BF16),
        pltpu.VMEM((NS, FH, 128), F32),
        pltpu.VMEM((2, 2, 4, 512, 128), F32),
        pltpu.VMEM((2, 2, 4, 512, 128), F32),
        pltpu.VMEM((128, 128), F32),
        pltpu.VMEM((128, 128), F32),
        pltpu.VMEM((5, 128, D), F32),
        pltpu.VMEM((4, 512, 128), BF16),
        pltpu.VMEM((3, 128, D), F32),
        pltpu.VMEM((S + 128, D), BF16),
        pltpu.VMEM((NS, 128), F32),
        pltpu.SemaphoreType.DMA((NS,)),
        pltpu.SemaphoreType.DMA((20,)),
        pltpu.SemaphoreType.DMA((NS,)),
        pltpu.SemaphoreType.DMA((NS,)),
    ]
    scratch += [pltpu.VMEM((2, 8, 128, 128), F32)] * 8
    scratch += [pltpu.VMEM((2, 8, 128, 128), BF16)] * 4
    scratch += [pltpu.VMEM((11, 64, 128), F32)] * 2
    scratch += [pltpu.VMEM((8, 128, 128), BF16)] * NS
    scratch += [pltpu.VMEM((6, 128, 128), BF16)] * 2
    scratch += [pltpu.VMEM((2, FH // 2, 128), F32)]
    return pl.pallas_call(
        _kernel,
        out_shape=jax.ShapeDtypeStruct((1, S, D), BF16),
        in_specs=[hbm] * 11,
        out_specs=hbm,
        scratch_shapes=scratch,
        compiler_params=pltpu.CompilerParams(vmem_limit_bytes=100 * 1024 * 1024),
    )(A_x, A_w_r.T, A_w_i.T, B_w_in.T, B_w_sp, B_b_sp.reshape(NS, 128), B_w_out,
      csm, cmat, ctw, zero)
```

```python
import functools
import math

import jax
import jax.numpy as jnp
import numpy as np
from jax import lax
import jax.experimental.pallas as pl
import jax.experimental.pallas.tpu as pltpu

S, D, F = 2048, 512, 1376
FH = F // 2
FHP = 768
NS = S // 128
F1 = 352
F2 = FH - F1
EPS = 1e-5
F32, BF16, U32 = jnp.float32, jnp.bfloat16, jnp.uint32
WP = 33
_NT = (((1,), (1,)), ((), ()))
_C1 = math.sqrt(2.0 / math.pi)
ALPHA = (0.044715 * _C1) ** (1.0 / 3.0)
GC = _C1 / ALPHA


@functools.lru_cache(maxsize=1)
def _tables():
    l = np.arange(128)
    kA = 2 * l
    kB = 2 * l + 1
    m0 = (l % 2) == 0
    kAs = kA[(l + 1) % 128]
    n1 = np.arange(128)[:, None].astype(np.float64)

    def cs(k):
        th = 2.0 * np.pi * ((n1 * k[None, :]) % D) / D
        return np.cos(th), np.sin(th)

    cA, sA = cs(kA)
    cAs, sAs = cs(kAs)
    cB, sB = cs(kB)
    F0 = np.where(m0[None, :], cA, -sAs)
    F2 = np.where(m0[None, :], -sAs, cA)
    sg = np.where(kB % 4 == 1, -1.0, 1.0)[None, :]
    zero_t = np.zeros((128, 128))
    cF = np.stack([F0, F2, cB, -sB - sg * cB, sg * sB - cB, zero_t]) / ALPHA

    wA = np.where(kA == 0, 1.0, 2.0)[None, :] / D
    wAs = np.where(kAs == 0, 1.0, 2.0)[None, :] / D
    G0 = np.where(m0[None, :], cA * wA, -sAs * wAs).T
    G0[127, :] = np.where(m0, 1.0, -1.0) / D
    G2 = np.where(m0[None, :], -sAs * wAs, cA * wA).T
    w2 = 2.0 / D
    tB = sg * sB
    cG = np.stack([G0, G2, (cB * w2).T, ((-tB - cB) * w2).T, ((tB - cB) * w2).T, zero_t])

    n2 = np.arange(64)[None, :]
    kh = np.arange(64)[:, None]
    Mf = np.zeros((32, 128, 128))
    for klo in range(32):
        ph = 2.0 * np.pi * ((n2 * (32 * kh + klo)) % S) / S
        c, s = np.cos(ph), np.sin(ph)
        Mf[klo] = np.block([[c, s], [-s, c]])
    Mi = np.transpose(Mf, (0, 2, 1)) / S
    cM = np.stack([Mf, Mi])

    a16 = np.arange(16)
    th16 = 2.0 * np.pi * ((a16[:, None] * a16[None, :]) % 16) / 16
    D16f = np.zeros((128, 128))
    D16f[0:16, :16] = np.cos(th16)
    D16f[16:32, :16] = -np.sin(th16)
    a128 = np.arange(128)
    th128 = 2.0 * np.pi * ((a128[:, None] * a128[None, :]) % 128) / 128
    cS = np.stack([D16f / ALPHA, D16f / S, np.cos(th128), np.sin(th128)])
    tht = 2.0 * np.pi * (a16[:, None] * a128[None, :]) / S
    tw = np.stack([np.cos(tht), np.sin(tht)])

    small = np.concatenate([cF, cG, cS], axis=0)
    return (small.astype(np.float32), cM.astype(np.float32), tw.astype(np.float32))


def _cadd(a, b):
    return (a[0] + b[0], a[1] + b[1])


def _csub(a, b):
    return (a[0] - b[0], a[1] - b[1])


def _dft4(y, sign):
    t0 = _cadd(y[0], y[2])
    t1 = _csub(y[0], y[2])
    t2 = _cadd(y[1], y[3])
    t3 = _csub(y[1], y[3])
    o0 = _cadd(t0, t2)
    o2 = _csub(t0, t2)
    if sign < 0:
        o1 = (t1[0] + t3[1], t1[1] - t3[0])
        o3 = (t1[0] - t3[1], t1[1] + t3[0])
    else:
        o1 = (t1[0] - t3[1], t1[1] + t3[0])
        o3 = (t1[0] + t3[1], t1[1] - t3[0])
    return [o0, o1, o2, o3]


def _ctw(a, num, den, sign):
    num = num % den
    if sign < 0:
        num = (den - num) % den
    if num == 0:
        return a
    if 4 * num == den:
        return (-a[1], a[0])
    if 2 * num == den:
        return (-a[0], -a[1])
    if 4 * num == 3 * den:
        return (a[1], -a[0])
    if (8 * num) % den == 0:
        r = math.sqrt(0.5)
        o = (8 * num) // den
        d = (a[0] - a[1])
        s = (a[0] + a[1])
        if o == 1:
            return (d * r, s * r)
        if o == 3:
            return (s * (-r), d * r)
        if o == 5:
            return (d * (-r), s * (-r))
        return (s * r, d * (-r))
    c = math.cos(2.0 * math.pi * num / den)
    s = math.sin(2.0 * math.pi * num / den)
    return (a[0] * c - a[1] * s, a[0] * s + a[1] * c)


def _dft8(x, sign):
    u = [_cadd(x[k], x[k + 4]) for k in range(4)]
    v = [_csub(x[k], x[k + 4]) for k in range(4)]
    ev = _dft4(u, sign)
    v1 = _ctw(v[1], 1, 8, sign)
    v3 = _ctw(v[3], 3, 8, sign)
    if sign < 0:
        t0 = (v[0][0] + v[2][1], v[0][1] - v[2][0])
        t1 = (v[0][0] - v[2][1], v[0][1] + v[2][0])
    else:
        t0 = (v[0][0] - v[2][1], v[0][1] + v[2][0])
        t1 = (v[0][0] + v[2][1], v[0][1] - v[2][0])
    t2 = _cadd(v1, v3)
    t3 = _csub(v1, v3)
    o1 = _cadd(t0, t2)
    o5 = _csub(t0, t2)
    if sign < 0:
        o3 = (t1[0] + t3[1], t1[1] - t3[0])
        o7 = (t1[0] - t3[1], t1[1] + t3[0])
    else:
        o3 = (t1[0] - t3[1], t1[1] + t3[0])
        o7 = (t1[0] + t3[1], t1[1] - t3[0])
    return [ev[0], o1, ev[1], o3, ev[2], o5, ev[3], o7]


def _gelu2a(xs):
    return xs * jnp.tanh(xs * (xs * xs + GC)) + xs


def _silu_h(hx):
    return hx * jnp.tanh(hx) + hx


def _dot(a, b):
    return jnp.dot(a, b, preferred_element_type=F32)


def _dot_nt(a, b):
    return lax.dot_general(a, b, _NT, preferred_element_type=F32)


def _rows(i, n):
    if isinstance(i, int):
        return pl.ds(i * n, n)
    return pl.ds(pl.multiple_of(i * n, n), n)


def _ds(start, n):
    if isinstance(start, int):
        return pl.ds(start, n)
    return pl.ds(pl.multiple_of(start, n), n)


def _kernel(x_hbm, wr_hbm, wi_hbm, win_hbm, wsp_hbm, bsp_hbm, wout_hbm,
            csm_hbm, cm_hbm, ctw_hbm, zero_hbm,
            out_hbm,
            xbuf, wint, csm, cmat, ctw, wbuf, wtr, wsp, wout, bspb, zsm,
            za_ref, z1_ref, y1_ref, zz_ref, xm_ref, um_ref,
            gate_ref, sbuf, obuf, bsp32,
            sem_x, sem_w, sem_sp, sem_o, *bufs):
    p1_refs, v_refs, yb_refs = bufs[0:4], bufs[4:8], bufs[8:12]
    zd_refs, lnb = bufs[12:16], bufs[16:32]
    hb_refs, gcar, tins = bufs[32:34], bufs[34], bufs[35:37]
    c_refs = dict(zip(("p", "11", "12", "21", "22"), bufs[37:42]))
    wa_ref, bop, zc_refs = bufs[42], bufs[43:49], bufs[49:53]
    hb_u = [r.bitcast(U32) for r in hb_refs]
    wa_u, bop_u = wa_ref.bitcast(U32), [r.bitcast(U32) for r in bop]
    lane = lax.broadcasted_iota(jnp.int32, (1, 128), 1)
    m0 = (lane & 1) == 0
    alt = jnp.where(m0, 1.0, -1.0).astype(F32)

    wint_u, csm_u, cmat_u = wint.bitcast(U32), csm.bitcast(U32), cmat.bitcast(U32)
    za_u, wout_u = za_ref.bitcast(U32), wout.bitcast(U32)
    lnb_u, tins_u = [r.bitcast(U32) for r in lnb], [r.bitcast(U32) for r in tins]
    yb_u = [r.bitcast(U32) for r in yb_refs]

    def _bf(v):
        return pltpu.bitcast(v, BF16)

    def cs(i):
        return _bf(csm_u[i])

    def x_copy(sig):
        return pltpu.make_async_copy(x_hbm.at[0, _rows(sig, 128), :],
                                     xbuf.at[_rows(sig, 128), :], sem_x.at[sig])

    def sp_copy(sig):
        return pltpu.make_async_copy(wsp_hbm.at[_rows(sig, 128), :],
                                     wsp.at[_rows(sig, 128), :], sem_sp.at[sig])

    def o_copy(sig):
        return pltpu.make_async_copy(obuf.at[_rows(sig, 128), :],
                                     out_hbm.at[0, _rows(sig, 128), :], sem_o.at[sig])

    c_win = [pltpu.make_async_copy(
        win_hbm.at[pl.ds((1 - h) * FH, FH), kd * 128:(kd + 1) * 128],
        wint.at[kd, pl.ds((1 - h) * FH, FH), :], sem_w.at[4 * h + kd])
        for h in range(2) for kd in range(4)]
    c_csf = pltpu.make_async_copy(csm_hbm.at[0:6], csm.at[0:6], sem_w.at[8])
    c_csr = pltpu.make_async_copy(csm_hbm.at[6:16], csm.at[6:16], sem_w.at[18])
    c_cm = pltpu.make_async_copy(cm_hbm, cmat, sem_w.at[9])
    c_tw = pltpu.make_async_copy(ctw_hbm, ctw, sem_w.at[10])
    c_bsp = pltpu.make_async_copy(bsp_hbm, bspb, sem_w.at[11])
    c_w = [pltpu.make_async_copy(w_hbm, wbuf.at[a], sem_w.at[12 + a])
           for a, w_hbm in enumerate((wr_hbm, wi_hbm))]
    c_wout = [pltpu.make_async_copy(wout_hbm.at[:, nt * 128:(nt + 1) * 128],
                                    wout.at[nt, 0:FH, :], sem_w.at[14 + nt])
              for nt in range(4)]
    c_zero = pltpu.make_async_copy(zero_hbm, zsm, sem_w.at[19])

    x_copy(0).start()
    c_zero.start()
    x_copy(4).start()
    for c in c_win[:4]:
        c.start()

    xm_ref[...] = jnp.zeros((128, 128), F32)
    wout[:, FH:FHP, :] = jnp.zeros((4, FHP - FH, 128), BF16)

    x_copy(0).wait()
    c_zero.wait()
    x_copy(4).wait()
    for c in c_win[4:]:
        c.start()
    x_copy(8).start()

    zero = zsm[0]
    never = jnp.full((8, 128), zero, jnp.int32) > 0

    pending = []

    def attach(p, vals, lo=0, hi=None):
        n = len(vals)
        if n == 0:
            return p
        nr = p.shape[0] // 8
        hi = nr if hi is None else hi
        at = {lo + ((u + 1) * (hi - lo)) // n - 1: vals[u] for u in range(n)}
        assert len(at) == n
        parts, r0 = [], 0
        for r in sorted(at):
            if r > r0:
                parts.append(p[r0 * 8:r * 8])
            parts.append(jnp.where(never, at[r], p[r * 8:(r + 1) * 8]))
            r0 = r + 1
        if r0 < nr:
            parts.append(p[r0 * 8:])
        return jnp.concatenate(parts, axis=0)

    def clobber(ref):
        junk = ref.shape[0] - 8
        ref[pl.ds(pl.multiple_of(junk + zero * 8, 8), 8), :] = jnp.zeros((8, 128), F32)

    def fenced(p, units, lo=0):
        return attach(p, [u() for u in units], lo)

    def drain(p, hi=None, lo=8):
        vals = [pltpu.bitcast(v, U32) for v in pending]
        del pending[:]
        return attach(p, vals, lo, hi)

    def ln_core(sig, rc, gate):
        xs = xbuf[pl.ds(sig * 128 + rc * 16, 16), :].astype(F32)
        if gate is not None:
            x00 = jnp.concatenate([jnp.where(never, gate, xs[0:8, 0:128]),
                                   jnp.where(never, gate, xs[8:16, 0:128])], axis=0)
            xs = jnp.concatenate([x00, xs[:, 128:]], axis=1)
        mu = jnp.sum(xs, axis=1, keepdims=True) * (1.0 / D)
        xc = xs - mu
        var = jnp.sum(xc * xc, axis=1, keepdims=True) * (1.0 / D)
        xn = xc * (lax.rsqrt(var + EPS) * ALPHA)
        x0, x1, x2, x3 = [xn[:, t * 128:(t + 1) * 128] for t in range(4)]
        s02 = x0 + x2
        s13 = x1 + x3
        a0 = s02 + s13
        r = pl.ds(rc * 16, 16)
        pp = x0 - x2
        q = x1 - x3
        for t, val in enumerate((a0, s02 - s13, pp, q, pp + q)):
            lnb[sig][4 + t, r, :] = val.astype(BF16)
        nyq = jnp.sum(a0 * alt, axis=1, keepdims=True)
        nyq = jnp.broadcast_to(nyq, (16, 128))
        pltpu.store(xm_ref.at[r, :], nyq,
                    mask=jnp.broadcast_to(lane == sig, (16, 128)))
        pending.append(nyq[0:8] + nyq[8:16])
        return x0, x1, x2, x3

    def ln_unit(sig, rc):
        def run(gate=None):
            for t, val in enumerate(ln_core(sig, rc, gate)):
                lnb[sig][t, pl.ds(rc * 16, 16), :] = val.astype(BF16)
        return run

    def bslot(sa):
        return 2 * (sa % 4 - 1) + sa // 4

    def lnp_unit(sa, rc):
        keep = {}

        def put(k, t, val):
            bop[bslot(sa)][2 * k + t, pl.ds(rc * 16, 16), :] = val.astype(BF16)

        def first(gate=None):
            xa = keep["xa"] = ln_core(sa, rc, gate)
            for t in range(2):
                put(1, t, xa[t])
                put(3, t, xa[2 + t] - xa[t])

        def second(gate=None):
            xa = keep["xa"]
            xb = ln_core(sa + 8, rc, gate)
            for t in range(2):
                b11, b21, b12, b22 = xa[t], xa[2 + t], xb[t], xb[2 + t]
                for k, val in ((0, b11 + b22), (2, b12 - b22), (4, b22), (5, b11 + b12),
                               (6, b21 + b22)):
                    put(k, t, val)
        return [first, second]

    _WA = {0: ((1, 0), (0, 1), 1), 1: ((0, 0), (0, 1), 1), 4: ((1, 0), (1, 1), 1),
           5: ((0, 0), (1, 0), -1), 6: ((1, 1), (0, 1), -1)}
    _WA_IDX = {k: i for i, k in enumerate(sorted(_WA))}

    def wa_unit(kind, t, ch):
        def run(gate):
            (ra, ka), (rb, kb), sign = _WA[kind]
            n = 8 if ch < 5 else 3
            au = wint_u[2 * ka + t, pl.ds(ra * (FH // 2) + ch * 64, 8 * n), :]
            au = jnp.where(jnp.full((n, 8, 128), zero, jnp.int32) > 0,
                           pltpu.bitcast(gate, U32), au.reshape(n, 8, 128))
            a = _bf(au.reshape(8 * n, 128)).astype(F32)
            b = _bf(wint_u[2 * kb + t, pl.ds(rb * (FH // 2) + ch * 64, 8 * n), :]).astype(F32)
            wa_ref[_WA_IDX[kind], t, pl.ds(ch * 128, 16 * n), :] = (
                a + b if sign > 0 else a - b).astype(BF16)
        return run

    def wa_units(kind):
        return [wa_unit(kind, t, ch) for t in range(2) for ch in range(6)]

    def release(p, units, lo=0, hi=FH // 8):
        for u, unit in enumerate(units):
            r = lo + (u * (hi - lo)) // len(units)
            unit(p[r * 8:r * 8 + 8])

    def wint_rows(r0, n):
        tiles = [wint_u[kd, pl.ds(r0 // 2, n // 2), :] for kd in range(4)]
        tiles[0] = drain(tiles[0], 30 if r0 == 0 else None)
        return jnp.concatenate([_bf(t) for t in tiles], axis=1)

    def xn_slab(sig):
        return jnp.concatenate([_bf(lnb_u[sig][t + zero]) for t in range(4)], axis=1)

    def z2_stream(sig, p):
        zd = zd_refs[sig // 4]
        c0 = s1 = s2 = None
        hist = []
        for i in range(11):
            n = 8 if i < 10 else 6
            v = p[i * 64:i * 64 + 8 * n]
            if i >= 2:
                v = jnp.concatenate([jnp.where(never, hist[i - 2][0], v[0:8]),
                                     jnp.where(never, hist[i - 2][1], v[8:16]),
                                     v[16:]], axis=0)
            y = _gelu2a(v).reshape(n, 8, 128)
            if i == 0:
                c0 = y[0]
            d = y - c0
            zd[4 * i:4 * i + n // 2] = d.reshape(n // 2, 16, 128)
            t1 = jnp.sum(d, axis=0)
            t2 = jnp.sum(d * d, axis=0)
            s1 = t1 if s1 is None else s1 + t1
            s2 = t2 if s2 is None else s2 + t2
            hist.append((s1, s2))
        ng = FH // 8
        mean_g = c0 + s1 * (1.0 / ng)
        mean = jnp.sum(mean_g, axis=0, keepdims=True) * 0.125
        dm = mean_g - mean
        m2 = s2 - s1 * s1 * (1.0 / ng) + dm * dm * float(ng)
        var = jnp.maximum(jnp.sum(m2, axis=0, keepdims=True) * (1.0 / FH), 0.0)
        rs = lax.rsqrt(var + EPS * (4.0 * ALPHA * ALPHA)) * (0.25 / ALPHA)
        rs = jnp.broadcast_to(rs, (8, 128))
        return rs, (c0 - mean) * rs

    nq1 = F1 // 16

    def put_za(kind, kt, q, val):
        za_ref[kind, kt, pl.ds(q * 16, 16), :] = val.reshape(16, 128).astype(BF16)

    def normp_units(sa, st_a, st_b):
        za_, zb_ = zd_refs[sa // 4], zd_refs[sa // 4 + 2]

        def unit(i):
            def run(gate):
                ra = jnp.where(never, gate, st_a[0])
                rb = jnp.where(never, gate, st_b[0])
                for q in (2 * i, 2 * i + 1):
                    a11 = za_[q + zero].reshape(2, 8, 128) * ra + st_a[1]
                    a12 = zb_[q + zero].reshape(2, 8, 128) * rb + st_b[1]
                    put_za(2, sa, q, a11)
                    put_za(4, sa, q, a11 + a12)
                    if q + nq1 < FH // 16:
                        a21 = za_[q + nq1 + zero].reshape(2, 8, 128) * ra + st_a[1]
                        a22 = zb_[q + nq1 + zero].reshape(2, 8, 128) * rb + st_b[1]
                        put_za(0, sa, q, a11 + a22)
                        put_za(1, sa, q, a21 + a22)
                        put_za(3, sa, q, a22)
                        put_za(5, sa, q, a21 - a11)
                        put_za(6, sa, q, a12 - a22)
                    else:
                        put_za(0, sa, q, a11)
                        put_za(6, sa, q, a12)
            return run
        return [unit(i) for i in range(11)]

    def z2_part(sig, units, extra=()):
        zd = zd_refs[sig // 4]
        p = _dot_nt(wint_rows(FH, FH), xn_slab(sig))
        release(p, units, 0, 64)
        release(p, extra)
        rs, sh = z2_stream(sig, p)
        kt = sig % 8

        def put(kind, q, val):
            put_za(kind, kt, q, val)

        def norm_unit(i):
            def run(gate):
                ri = jnp.where(never, gate, rs)
                for q in (2 * i, 2 * i + 1):
                    has2 = q + nq1 < FH // 16
                    top = zd[q + zero].reshape(2, 8, 128) * ri + sh
                    bot = (zd[q + nq1 + zero].reshape(2, 8, 128) * ri + sh) if has2 else None
                    if sig < 8:
                        zd[q] = top.reshape(16, 128)
                        put(2, q, top)
                        if has2:
                            zd[q + nq1] = bot.reshape(16, 128)
                            put(5, q, bot - top)
                    else:
                        zp = zd_refs[sig // 4 - 2]
                        a11 = zp[q + zero].reshape(2, 8, 128)
                        put(4, q, a11 + top)
                        if has2:
                            a21 = zp[q + nq1 + zero].reshape(2, 8, 128)
                            put(0, q, a11 + bot)
                            put(1, q, a21 + bot)
                            put(3, q, bot)
                            put(6, q, top - bot)
                        else:
                            put(0, q, a11)
                            put(6, q, top)
            return run
        return [norm_unit(i) for i in range(11)]

    def z1_part(sig, ln_units, norm_units, extra=()):
        p = _dot_nt(wint_rows(0, FH), xn_slab(sig))
        release(p, ln_units, 0, 64)
        release(p, norm_units, 8)
        release(p, extra)
        z1_ref[sig] = _gelu2a(p)

    def zprod(kind, sa, hard=None):
        if kind == 2:
            tiles = [wint_u[t, pl.ds(FH // 2, FH // 2), :] for t in range(2)]
        elif kind == 3:
            tiles = [wint_u[2 + t, pl.ds(0, FH // 2), :] for t in range(2)]
        else:
            tiles = [wa_u[_WA_IDX[kind] + zero, t] for t in range(2)]
        if hard is not None:
            tiles[0] = drain(tiles[0], hard[1], hard[0])
        rhs = jnp.concatenate([_bf(bop_u[bslot(sa)][2 * kind + t + zero]) for t in range(2)],
                              axis=1)
        return _dot_nt(jnp.concatenate([_bf(t) for t in tiles], axis=1), rhs)

    class ZPair:
        def __init__(self, sa, k):
            self.sa = sa
            self.c11, self.c22 = zc_refs[2 * k], zc_refs[2 * k + 1]

        def r1(self, lnu=(), units=(), hard=None):
            m4 = zprod(3, self.sa, hard)
            m2 = zprod(1, self.sa)
            release(m4, lnu, 0, 50)
            release(m4, units, 4)
            z1_ref[self.sa] = _gelu2a(m2 + m4)
            self.c11[0:FH, :] = m4
            self.c22[0:FH, :] = m2
            clobber(self.c11)
            clobber(self.c22)

        def r2(self, lnu=(), units=(), hard=None):
            m5 = zprod(4, self.sa, hard)
            m3 = zprod(2, self.sa)
            release(m5, lnu, 0, 50)
            release(m5, units, 4)
            self.st_b = z2_stream(self.sa + 8, m3 + m5)
            self.c11[0:FH, :] = self.c11[0:FH, :] - m5
            self.c22[0:FH, :] = m3 - self.c22[0:FH, :]
            clobber(self.c11)
            clobber(self.c22)

        def r3(self, lnu=(), units=(), hard=None):
            m7 = zprod(6, self.sa, hard)
            m1 = zprod(0, self.sa)
            release(m7, lnu, 0, 50)
            release(m7, units, 4)
            self.st_a = z2_stream(self.sa, self.c11[0:FH, :] + (m1 + m7))
            self.c22[0:FH, :] = self.c22[0:FH, :] + m1
            clobber(self.c22)

        def r4(self, lnu=(), units=(), hard=None):
            m6 = zprod(5, self.sa, hard)
            release(m6, lnu, 0, 50)
            release(m6, units, 4)
            z1_ref[self.sa + 8] = _gelu2a(self.c22[0:FH, :] + m6)

        def norms(self):
            return normp_units(self.sa, self.st_a, self.st_b)

    def d_fwd(j, lnu=()):
        def lhs(t, h):
            return jnp.concatenate(
                [_bf(lnb_u[j + 4 * b][t + zero, pl.ds(rc * 8, 8), :])
                 for rc in (2 * h, 2 * h + 1) for b in range(4)], axis=0)
        res = [[_dot(lhs(t, h), cs(i)) for i, t in enumerate((4, 5, 8, 6, 7))]
               for h in range(4)]
        t0, t2, k1, k2, k3 = [jnp.concatenate([res[h][i] for h in range(4)], axis=0)
                              for i in range(5)]
        release(t0, lnu, 0, 40)
        for rc in range(16):
            for c in range(2):
                g = []
                for b in range(4):
                    r0 = (rc // 2) * 64 + b * 16 + (rc % 2) * 8
                    if c == 0:
                        t0c = t0[r0:r0 + 8]
                        t2c = t2[r0:r0 + 8]
                        g.append((jnp.where(m0, t0c, t2c),
                                  pltpu.roll(jnp.where(m0, t2c, t0c), 1, 1)))
                    else:
                        k1c = k1[r0:r0 + 8]
                        g.append((k1c + k3[r0:r0 + 8], k2[r0:r0 + 8] - k1c * alt))
                o = _dft4(g, -1)
                if c == 0:
                    pending.append(o[0][1])
                r = pl.ds(j * 128 + rc * 8, 8)
                for e in range(4):
                    y1_ref[c, 0, e, r, :] = o[e][0]
                    y1_ref[c, 1, e, r, :] = o[e][1]

    for rc in range(8):
        ln_unit(0, rc)()
        ln_unit(4, rc)()
    del pending[:]
    for c in c_win[:4]:
        c.wait()
    for sig in (12, 1, 9):
        x_copy(sig).start()
    c_csf.start()

    def lns(sig):
        return [ln_unit(sig, rc) for rc in range(8)]

    class Halves:
        def __init__(self, units):
            self.units = units

        def __getitem__(self, sl):
            return [h for u in self.units[sl] for h in u]

    def lnps(sa):
        return Halves([lnp_unit(sa, rc) for rc in range(8)])

    wk = {k: wa_units(k) for k in _WA}
    norms0 = z2_part(0, [], wk[4][:6])
    norms4 = z2_part(4, [], wk[4][6:])
    for c in c_win[4:]:
        c.wait()
    x_copy(8).wait()
    rest = (5, 13, 2, 10, 6, 14, 3, 11, 7, 15)
    for sig in rest:
        x_copy(sig).start()
    z1_part(0, lns(8), norms0, wk[1][:4])
    z1_part(4, [], norms4, wk[1][4:])
    for s2 in (12, 1, 9):
        x_copy(s2).wait()
    c_csf.wait()
    for s2 in (0, 8, 2, 10):
        sp_copy(s2).start()
    for c in c_w + [c_cm, c_bsp] + c_wout + [c_tw, c_csr]:
        c.start()
    nxt = lnps(1)
    norms8 = z2_part(8, lns(12))
    z1_part(8, nxt[:3], norms8, wk[6][:4])
    d_fwd(0)
    norms12 = z2_part(12, nxt[3:], wk[6][4:6])
    z1_part(12, [], norms12, wk[6][6:])
    for s2 in rest:
        x_copy(s2).wait()
    prev = []
    lb = lnps(5)
    for j in range(1, 4):
        za_p, zb_p = ZPair(j, 0), ZPair(j + 4, 1)
        one = j == 1
        nxa = lnps(j + 1) if j < 3 else Halves([])
        nxb = lnps(j + 5) if j < 3 else Halves([])
        k = 0 if one else 2
        za_p.r1(lb[k:k + 4] if not one else lb[0:5], wk[0][:6] if one else [])
        za_p.r2(lb[k + 4:] if not one else lb[5:], wk[0][6:] if one else prev[:4])
        za_p.r3((), prev[4:], (8, 30))
        zb_p.r1(nxa[:1], za_p.norms())
        d_fwd(j, nxa[1:3])
        zb_p.r2(nxa[3:5], wk[5][:6] if one else [], (8, 40))
        zb_p.r3(nxa[5:], wk[5][6:] if one else [])
        prev = zb_p.norms()
        za_p.r4(nxb[:2], prev if j == 3 else [], (8, 30))
        zb_p.r4()
        lb = nxb

    _RHS = {0: ((0, 0, 1), (1, 1, 1)), 1: ((0, 0, 1),), 2: ((1, 0, 1), (1, 1, -1)),
            3: ((0, 1, 1), (0, 0, -1)), 4: ((1, 1, 1),), 5: ((0, 0, 1), (1, 0, 1)),
            6: ((0, 1, 1), (1, 1, 1))}
    _OUT = {0: (("11", 1), ("22", 1)), 1: (("21", 1), ("22", -1)),
            2: (("12", 1), ("22", 1)), 3: (("11", 1), ("21", 1)),
            4: (("11", -1), ("12", 1)), 5: (("22", 1),), 6: (("11", 1),)}

    class Pair:
        def __init__(self, s1):
            self.s = (s1, s1 + 8)
            self.c = {}
            self.neg = set()
            self.part = None

        def p(self, m, kp, units=(), lo=0, hard=False):
            rows = F2 if m in (1, 3, 5) else F1
            tiles = [za_u[m, 4 * kp + t, 0:rows // 2, :] for t in range(4)]
            if hard:
                tiles[0] = drain(tiles[0], 20, 2)
            lhs = jnp.concatenate([_bf(t) for t in tiles], axis=1)
            blk = [wsp[_rows(self.s[th], 128), pl.ds(sh * 1024 + kp * 512, 512)]
                   for th, sh, _ in _RHS[m]]
            if len(blk) == 1:
                rhs = blk[0]
            else:
                a, b = blk[0].astype(F32), blk[1].astype(F32)
                rhs = (a + b if _RHS[m][1][2] > 0 else a - b).astype(BF16)
            p = _dot_nt(lhs, rhs)
            self.mid = p[200:208]
            p = fenced(p, list(units), lo)
            if kp == 0:
                c_refs["p"][0:rows, :] = p
                clobber(c_refs["p"])
                return
            p = c_refs["p"][0:rows, :] + p
            for name, sign in _OUT[m]:
                ref = c_refs[name]
                n = F1 if name[0] == "1" else F2
                k = min(n, rows)
                if name in self.neg:
                    assert sign > 0 and k == n
                    self.neg.remove(name)
                    ref[0:k, :] = p[0:k] - ref[0:k, :]
                elif name not in self.c:
                    if sign < 0:
                        self.neg.add(name)
                    ref[0:k, :] = p[0:k]
                    if k < n:
                        ref[k:n, :] = jnp.zeros((n - k, 128), F32)
                elif sign > 0:
                    ref[0:k, :] = ref[0:k, :] + p[0:k]
                else:
                    ref[0:k, :] = ref[0:k, :] - p[0:k]
                self.c[name] = True
                clobber(ref)

        def both(self, m, u0=(), u1=()):
            self.p(m, 0, u0)
            self.p(m, 1, u1)

        def acc(self, which):
            return c_acc(which)

    def c_acc(which):
        a, b = ("11", "21") if which == 0 else ("12", "22")
        return jnp.concatenate([c_refs[a][0:F1, :], c_refs[b][0:F2, :]], axis=0)

    def h_tiles(sig, acc, slot):
        bias = bsp32[pl.ds(sig, 1), :]
        for t in range(6):
            n = 128 if t < 5 else FH - 640
            ht = z1_ref[sig, pl.ds(t * 128, n), :] * (acc[t * 128:t * 128 + n] + bias)
            if n < 128:
                ht = jnp.concatenate([ht, jnp.zeros((128 - n, 128), F32)], axis=0)
            ht = ht.astype(BF16).T
            hb_refs[slot][t] = ht
            pending.append(pltpu.bitcast(ht[112:128], F32))

    def small(slot, after=None, units=()):
        tiles = [hb_u[slot][t + zero] for t in range(6)]
        if after is not None:
            tiles[0] = attach(tiles[0], [pltpu.bitcast(after.mid, U32)], 0, 1)
        h = jnp.concatenate([_bf(t) for t in tiles], axis=1)
        wo = jnp.concatenate([_bf(wout_u[nt]) for nt in range(4)], axis=1)
        bo = _dot(h, wo)
        if units:
            n = len(units)
            bo = jnp.concatenate(
                [fenced(bo[:, nt * 128:(nt + 1) * 128], units[nt * n // 4:(nt + 1) * n // 4])
                 for nt in range(4)], axis=1)
        return _silu_h(bo)

    def save_acc(acc):
        gcar[0] = acc[0:FH // 2]
        gcar[1] = acc[FH // 2:FH]

    def load_acc():
        return jnp.concatenate([gcar[zero], gcar[1 + zero]], axis=0)

    def f_unit(c, e, rc):
        def run():
            xs = []
            for a in range(8):
                r = pl.ds(a * 64 + rc * 8, 8)
                xs.append(_ctw((y1_ref[c + zero, 0, e, r, :], y1_ref[c + zero, 1, e, r, :]),
                               a * e, 32, -1))
            o = _dft8(xs, -1)
            for cc in range(8):
                p1_refs[e][c, cc, pl.ds(rc * 8, 8), :] = o[cc][0]
                p1_refs[e][c, cc, pl.ds(64 + rc * 8, 8), :] = o[cc][1]
            return o[7][1]
        return run

    def f_units(e):
        return [f_unit(c, e, rc) for c in range(2) for rc in range(8)]

    def w_unit(a, kb):
        def run():
            wt = pltpu.bitcast(wbuf[a, 0:256, kb * 128:(kb + 1) * 128], U32).T
            for h in range(4):
                wtr[a, pl.ds((4 * kb + h) * WP, 32), :] = wt[h * 32:(h + 1) * 32]
            return pltpu.bitcast(wt[120:128], F32)
        return run

    def mid1(e):
        for cc in range(8):
            klo = e + 4 * cc
            wru = wtr[0, pl.ds(klo, 64, stride=WP), :]
            wiu = wtr[1, pl.ds(klo, 64, stride=WP), :]
            for c in range(2):
                if c == 0:
                    wr = pltpu.bitcast(wru << 16, F32)
                    wi = pltpu.bitcast(wiu << 16, F32)
                else:
                    wr = pltpu.bitcast(wru & jnp.uint32(0xFFFF0000), F32)
                    wi = pltpu.bitcast(wiu & jnp.uint32(0xFFFF0000), F32)
                xh = _dot(_bf(cmat_u[0, klo]), p1_refs[e][c + zero, cc].astype(BF16))
                xr, xi = xh[0:64], xh[64:128]
                yb_refs[e][c, cc, 0:64, :] = (xr * wr - xi * wi).astype(BF16)
                yb_refs[e][c, cc, 64:128, :] = (xr * wi + xi * wr).astype(BF16)

    def mid2(e, units=()):
        n = len(units)
        for cc in range(8):
            klo = e + 4 * cc
            for c in range(2):
                k = 2 * cc + c
                v = _dot(_bf(cmat_u[1, klo]), _bf(yb_u[e][c + zero, cc]))
                v_refs[e][c, cc] = fenced(v, units[k * n // 16:(k + 1) * n // 16])

    def i_unit(c, e, rc):
        def run():
            xs = []
            for cc in range(8):
                xs.append((v_refs[e][c + zero, cc, pl.ds(rc * 8, 8), :],
                           v_refs[e][c + zero, cc, pl.ds(64 + rc * 8, 8), :]))
            o = _dft8(xs, +1)
            for a in range(8):
                t = _ctw(o[a], a * e, 32, +1)
                r = pl.ds(a * 64 + rc * 8, 8)
                zz_ref[c, 0, e, r, :] = t[0]
                zz_ref[c, 1, e, r, :] = t[1]
            return t[1]
        return run

    def i_units(e):
        return [i_unit(c, e, rc) for c in range(2) for rc in range(8)]

    nq = {}

    def nyq0():
        twc, tws = ctw[0], ctw[1]
        aa = _dot_nt(_bf(csm_u[12, 0:16, :]), xm_ref[...].astype(BF16))
        ar, ai = aa[0:16], aa[16:32]
        nq[0] = jnp.concatenate([ar * twc + ai * tws, ai * twc - ar * tws], axis=0)

    def nyq1():
        l16 = lax.broadcasted_iota(jnp.int32, (16, 128), 1)
        r16 = lax.broadcasted_iota(jnp.int32, (16, 128), 0)
        idx = 16 * (l16 & 7) + r16
        grp = l16 >> 3
        wn = []
        for a in range(2):
            wrow = wbuf[a, 256:257, :].astype(F32)
            acc = jnp.zeros((16, 128), F32)
            for ka in range(16):
                rowb = jnp.broadcast_to(wrow[:, ka * 128:(ka + 1) * 128], (16, 128))
                acc = jnp.where(grp == ka, jnp.take_along_axis(rowb, idx, axis=1), acc)
            wn.append(acc)
        cs128 = jnp.concatenate([cs(14), cs(15)], axis=1)
        p = _dot(nq[0].astype(BF16), cs128)
        xr = p[0:16, 0:128] + p[16:32, 128:256]
        xi = p[16:32, 0:128] - p[0:16, 128:256]
        nq[1] = jnp.concatenate([xr * wn[0] - xi * wn[1], xr * wn[1] + xi * wn[0]], axis=0)

    def nyq2():
        twc, tws = ctw[0], ctw[1]
        cs128 = jnp.concatenate([cs(14), cs(15)], axis=1)
        p = _dot(nq[1].astype(BF16), cs128)
        vr = p[0:16, 0:128] - p[16:32, 128:256]
        vi = p[16:32, 0:128] + p[0:16, 128:256]
        nq[2] = jnp.concatenate([vr * twc - vi * tws, vi * twc + vr * tws,
                                 jnp.zeros((96, 128), F32)], axis=0)

    def nyq3():
        um_ref[...] = _dot(nq[2].T.astype(BF16), cs(13))

    for c in (c_wout + c_w + [c_cm, c_tw, c_bsp, c_csr]
              + [sp_copy(sig) for sig in (0, 8, 2, 10)]):
        c.wait()
    for sig in (4, 12, 1, 9, 5, 13, 6, 14, 3, 11, 7, 15):
        sp_copy(sig).start()
    bsp32[...] = bspb[...].astype(F32) * (0.25 / ALPHA)
    wu = [w_unit(a, kb) for kb in range(NS) for a in range(2)]
    fu = [f_units(e) for e in range(4)]
    iu = [i_units(e) for e in range(4)]
    pa, pb = Pair(0), Pair(2)

    def mix(a, b):
        out = []
        for k in range(max(len(a), len(b))):
            out += a[k:k + 1] + b[k:k + 1]
        return out

    pa.p(3, 0, mix(fu[0][0:4], wu[0:4]))
    pa.p(3, 1, mix(fu[0][4:8], wu[4:8]))
    pa.p(1, 0, mix(fu[0][8:16], wu[8:14]))
    pa.p(1, 1, mix(fu[1][0:6], wu[14:20]))
    pa.p(6, 0, mix(fu[1][6:9], wu[20:26]))
    pa.p(6, 1, mix(fu[1][9:12], wu[26:32]))
    nyq0()
    pa.p(4, 0, fu[1][12:16])
    mid1(0)
    pa.p(4, 1, fu[2][0:6])
    mid2(0, fu[2][6:16])
    pa.p(0, 0, iu[0][0:4])
    mid1(1)
    pa.p(0, 1, iu[0][4:8])
    h_tiles(0, pa.acc(0), 0)
    nyq1()
    mid2(1, iu[0][8:16] + fu[3][0:6])
    pa.p(2, 0, fu[3][6:9], 0, True)
    gate_ref[0] = small(0, pa, fu[3][9:16] + iu[1][0:8])
    pa.p(2, 1, iu[1][8:12])
    mid1(2)
    pa.p(5, 0, iu[1][12:16])
    mid2(2)
    nyq2()
    pa.p(5, 1, iu[2][0:4])
    h_tiles(8, pa.acc(1), 1)
    mid1(3)
    pb.p(3, 0, iu[2][4:8], 0, True)
    gate_ref[1] = small(1, pb, iu[2][8:16])
    mid2(3)
    nyq3()
    pb.p(3, 1, iu[3][0:4])
    pb.both(1, iu[3][4:12], iu[3][12:16])
    pb.both(6)
    pb.both(4)
    pb.both(0)
    h_tiles(2, pb.acc(0), 0)
    pb.p(2, 0)
    pb.p(2, 1, hard=True)
    gate_ref[2] = small(0, pb)
    pb.both(5)
    sbuf[5] = jnp.zeros((128, D), F32)

    def emit(sig, rc, sv, g, dst=None):
        r = _ds(sig * 128 + rc * 16, 16)
        ro = r if dst is None else _ds(dst * 128 + rc * 16, 16)
        obuf[ro, :] = (xbuf[r, :].astype(F32) + sv * g).astype(BF16)

    def finish(sig, slot, g, dst=None):
        for rc in range(8):
            emit(sig, rc, sbuf[slot + zero, pl.ds(rc * 16, 16), :],
                 g[rc * 16:(rc + 1) * 16], dst)

    def r_units(j, tb):
        tin = tins[tb]

        def r_unit(c, rc):
            def run():
                r = _ds(j * 128 + rc * 16, 16)
                u = _dft4([(zz_ref[c, 0, e, r, :], zz_ref[c, 1, e, r, :])
                           for e in range(4)], +1)
                for b in range(4):
                    ro = pl.ds(rc * 64 + b * 16, 16)
                    re, im = u[b]
                    if c == 0:
                        nq_col = pltpu.roll(um_ref[pl.ds(rc * 16, 16), :],
                                            (128 - 4 * b - j) % 128, 1)
                        ip = pltpu.roll(jnp.where(lane == 0, nq_col, im), 127, 1)
                        tin[0, ro, :] = jnp.where(m0, re, ip).astype(BF16)
                        tin[1, ro, :] = jnp.where(m0, ip, re).astype(BF16)
                    else:
                        im = im * alt
                        tin[2, ro, :] = (re + im).astype(BF16)
                        tin[3, ro, :] = re.astype(BF16)
                        tin[4, ro, :] = im.astype(BF16)
                return ip[8:16] if c == 0 else u[3][1][8:16]
            return run
        return [r_unit(c, rc) for rc in range(8) for c in range(2)]

    def d_inv(j, tb, sink):
        tin_u = tins_u[tb]
        res = [[_dot(_bf(tin_u[i + zero, pl.ds(h * 64, 64), :]), cs(6 + i)) for i in range(5)]
               for h in range(4)]
        b0, b2, k1, k2, k3 = [jnp.concatenate([res[h][i] for h in range(4)], axis=0)
                              for i in range(5)]
        for rc in range(8):
            for b in range(4):
                r0 = rc * 64 + b * 16
                b0c = b0[r0:r0 + 16]
                b2c = b2[r0:r0 + 16]
                pc = k1[r0:r0 + 16] + k3[r0:r0 + 16]
                qc = k1[r0:r0 + 16] + k2[r0:r0 + 16]
                e02 = b0c + b2c
                o02 = b0c - b2c
                sink(b, rc, jnp.concatenate([e02 + pc, o02 - qc, e02 - pc, o02 + qc], axis=1))

    def phase3(i, carry):
        j0, j1 = 2 * i, 2 * i + 1
        for d in (4, 12, 1, 9, 5, 13):
            sp_copy(j0 + d).wait()

        def sink0(b, rc, sv):
            if b % 2 == 0:
                emit(j0 + 4 * b, rc, sv, gate_ref[j0 + b // 2, pl.ds(rc * 16, 16), :])
            else:
                sbuf[b // 2, pl.ds(rc * 16, 16), :] = sv

        def sink1(b, rc, sv):
            sbuf[2 + b, pl.ds(rc * 16, 16), :] = sv

        def done(sig, slot, g):
            finish(sig, slot, g)
            o_copy(sig).start()

        first = i == 0
        car = jnp.where(first, 10, 13)
        qa, qb, qc = Pair(j0 + 4), Pair(j1), Pair(j1 + 4)
        r0, r1 = r_units(j0, 0), r_units(j1, 1)
        h_tiles(car, c_acc(1), 1)
        qa.p(3, 0, r0[:8])
        qa.p(3, 1, r0[8:], 0, True)
        g = small(1, qa)
        gate_ref[jnp.where(first, 3, 4)] = g
        finish(car, 5, g, jnp.where(first, NS, car))
        qa.p(1, 0)
        d_inv(j0, 0, sink0)
        o_copy(j0).start()
        o_copy(j0 + 8).start()
        qa.p(1, 1)
        qa.both(6)
        qa.both(4)
        qa.both(0)
        h_tiles(j0 + 4, qa.acc(0), 0)
        qa.p(2, 0)
        qa.p(2, 1, hard=True)
        done(j0 + 4, 0, small(0, qa))
        qa.both(5, r1[:8], r1[8:])
        h_tiles(j0 + 12, qa.acc(1), 1)
        qb.p(3, 0)
        qb.p(3, 1, hard=True)
        done(j0 + 12, 1, small(1, qb))
        d_inv(j1, 1, sink1)
        qb.both(1)
        qb.both(6)
        qb.both(4)
        qb.both(0)
        h_tiles(j1, qb.acc(0), 0)
        qb.p(2, 0)
        qb.p(2, 1, hard=True)
        done(j1, 2, small(0, qb))
        qb.both(5)
        h_tiles(j1 + 8, qb.acc(1), 1)
        qc.p(3, 0)
        qc.p(3, 1, hard=True)
        done(j1 + 8, 4, small(1, qc))
        qc.both(1)
        qc.both(6)
        qc.both(4)
        qc.both(0)
        h_tiles(j1 + 4, qc.acc(0), 0)
        qc.p(2, 0)
        qc.p(2, 1, hard=True)
        done(j1 + 4, 3, small(0, qc))
        qc.both(5)

        @pl.when(i > 0)
        def _():
            o_copy(13).start()
        return carry

    lax.fori_loop(0, 2, phase3, 0)
    ht = z1_ref[NS - 1] * (c_acc(1) + bsp32[NS - 1:NS, :])
    ht = jnp.concatenate([ht, jnp.zeros((FHP - FH, 128), F32)], axis=0).astype(BF16)
    wo = jnp.concatenate([_bf(wout_u[nt]) for nt in range(4)], axis=1)
    finish(NS - 1, 5, _silu_h(_dot(ht.T, wo)))
    o_copy(NS - 1).start()
    for sig in range(NS):
        o_copy(sig).wait()


@jax.jit
def pallas_recurrent_scan__spectral_gfnet__mixer_gmlp__prompt_kernel(
    A_x: jax.Array,
    A_w_r: jax.Array,
    A_w_i: jax.Array,
    B_x: jax.Array,
    B_w_in: jax.Array,
    B_w_sp: jax.Array,
    B_b_sp: jax.Array,
    B_w_out: jax.Array,
):
    del B_x
    small, cm, tw = _tables()
    csm = jnp.asarray(small, dtype=BF16)
    cmat = jnp.asarray(cm, dtype=BF16)
    ctw = jnp.asarray(tw, dtype=F32)
    zero = jnp.zeros((1,), jnp.int32)
    hbm = pl.BlockSpec(memory_space=pltpu.HBM)
    scratch = [
        pltpu.VMEM((S, D), BF16),
        pltpu.VMEM((4, F, 128), BF16),
        pltpu.VMEM((16, 128, 128), BF16),
        pltpu.VMEM((2, 32, 128, 128), BF16),
        pltpu.VMEM((2, 16, 128), F32),
        pltpu.VMEM((2, D // 2 + 1, S), BF16),
        pltpu.VMEM((2, 64 * WP, 128), U32),
        pltpu.VMEM((S, S), BF16),
        pltpu.VMEM((4, FHP, 128), BF16),
        pltpu.VMEM((NS, 128), BF16),
        pltpu.SMEM((1,), jnp.int32),
        pltpu.VMEM((7, 8, F1, 128), BF16),
        pltpu.VMEM((NS, FH, 128), F32),
        pltpu.VMEM((2, 2, 4, 512, 128), F32),
        pltpu.VMEM((2, 2, 4, 512, 128), F32),
        pltpu.VMEM((128, 128), F32),
        pltpu.VMEM((128, 128), F32),
        pltpu.VMEM((5, 128, D), F32),
        pltpu.VMEM((6, 128, D), F32),
        pltpu.VMEM((S + 128, D), BF16),
        pltpu.VMEM((NS, 128), F32),
        pltpu.SemaphoreType.DMA((NS,)),
        pltpu.SemaphoreType.DMA((20,)),
        pltpu.SemaphoreType.DMA((NS,)),
        pltpu.SemaphoreType.DMA((NS,)),
    ]
    scratch += [pltpu.VMEM((2, 8, 128, 128), F32)] * 8
    scratch += [pltpu.VMEM((2, 8, 128, 128), BF16)] * 4
    scratch += [pltpu.VMEM((FH // 16, 16, 128), F32)] * 4
    scratch += [pltpu.VMEM((9, 128, 128), BF16)] * NS
    scratch += [pltpu.VMEM((6, 128, 128), BF16)] * 2
    scratch += [pltpu.VMEM((2, FH // 2, 128), F32)]
    scratch += [pltpu.VMEM((5, 512, 128), BF16)] * 2
    scratch += [pltpu.VMEM((F1 + 8, 128), F32)] * 5
    scratch += [pltpu.VMEM((5, 2, FH, 128), BF16)]
    scratch += [pltpu.VMEM((14, 128, 128), BF16)] * 6
    scratch += [pltpu.VMEM((FH + 8, 128), F32)] * 4
    return pl.pallas_call(
        _kernel,
        out_shape=jax.ShapeDtypeStruct((1, S, D), BF16),
        in_specs=[hbm] * 11,
        out_specs=hbm,
        scratch_shapes=scratch,
        compiler_params=pltpu.CompilerParams(vmem_limit_bytes=100 * 1024 * 1024),
    )(A_x, A_w_r.T, A_w_i.T, B_w_in.T, B_w_sp, B_b_sp.reshape(NS, 128), B_w_out,
      csm, cmat, ctw, zero)
```

```python
import functools
import math

import jax
import jax.numpy as jnp
import numpy as np
from jax import lax
import jax.experimental.pallas as pl
import jax.experimental.pallas.tpu as pltpu

S, D, F = 2048, 512, 1376
FH = F // 2
FHP = 768
NS = S // 128
F1 = 352
F2 = FH - F1
EPS = 1e-5
F32, BF16, U32 = jnp.float32, jnp.bfloat16, jnp.uint32
WP = 33
_NT = (((1,), (1,)), ((), ()))
_C1 = math.sqrt(2.0 / math.pi)
ALPHA = (0.044715 * _C1) ** (1.0 / 3.0)
GC = _C1 / ALPHA


@functools.lru_cache(maxsize=1)
def _tables():
    l = np.arange(128)
    kA = 2 * l
    kB = 2 * l + 1
    m0 = (l % 2) == 0
    kAs = kA[(l + 1) % 128]
    n1 = np.arange(128)[:, None].astype(np.float64)

    def cs(k):
        th = 2.0 * np.pi * ((n1 * k[None, :]) % D) / D
        return np.cos(th), np.sin(th)

    cA, sA = cs(kA)
    cAs, sAs = cs(kAs)
    cB, sB = cs(kB)
    F0 = np.where(m0[None, :], cA, -sAs)
    F2 = np.where(m0[None, :], -sAs, cA)
    sg = np.where(kB % 4 == 1, -1.0, 1.0)[None, :]
    zero_t = np.zeros((128, 128))
    cF = np.stack([F0, F2, cB, -sB - sg * cB, sg * sB - cB, zero_t]) / ALPHA

    wA = np.where(kA == 0, 1.0, 2.0)[None, :] / D
    wAs = np.where(kAs == 0, 1.0, 2.0)[None, :] / D
    G0 = np.where(m0[None, :], cA * wA, -sAs * wAs).T
    G0[127, :] = np.where(m0, 1.0, -1.0) / D
    G2 = np.where(m0[None, :], -sAs * wAs, cA * wA).T
    w2 = 2.0 / D
    tB = sg * sB
    cG = np.stack([G0, G2, (cB * w2).T, ((-tB - cB) * w2).T, ((tB - cB) * w2).T, zero_t])

    n2 = np.arange(64)[None, :]
    kh = np.arange(64)[:, None]
    Mf = np.zeros((32, 128, 128))
    for klo in range(32):
        ph = 2.0 * np.pi * ((n2 * (32 * kh + klo)) % S) / S
        c, s = np.cos(ph), np.sin(ph)
        Mf[klo] = np.block([[c, s], [-s, c]])
    Mi = np.transpose(Mf, (0, 2, 1)) / S
    cM = np.stack([Mf, Mi])

    a16 = np.arange(16)
    th16 = 2.0 * np.pi * ((a16[:, None] * a16[None, :]) % 16) / 16
    D16f = np.zeros((128, 128))
    D16f[0:16, :16] = np.cos(th16)
    D16f[16:32, :16] = -np.sin(th16)
    a128 = np.arange(128)
    th128 = 2.0 * np.pi * ((a128[:, None] * a128[None, :]) % 128) / 128
    cS = np.stack([D16f / ALPHA, D16f / S, np.cos(th128), np.sin(th128)])
    tht = 2.0 * np.pi * (a16[:, None] * a128[None, :]) / S
    tw = np.stack([np.cos(tht), np.sin(tht)])

    small = np.concatenate([cF, cG, cS], axis=0)
    return (small.astype(np.float32), cM.astype(np.float32), tw.astype(np.float32))


def _cadd(a, b):
    return (a[0] + b[0], a[1] + b[1])


def _csub(a, b):
    return (a[0] - b[0], a[1] - b[1])


def _dft4(y, sign):
    t0 = _cadd(y[0], y[2])
    t1 = _csub(y[0], y[2])
    t2 = _cadd(y[1], y[3])
    t3 = _csub(y[1], y[3])
    o0 = _cadd(t0, t2)
    o2 = _csub(t0, t2)
    if sign < 0:
        o1 = (t1[0] + t3[1], t1[1] - t3[0])
        o3 = (t1[0] - t3[1], t1[1] + t3[0])
    else:
        o1 = (t1[0] - t3[1], t1[1] + t3[0])
        o3 = (t1[0] + t3[1], t1[1] - t3[0])
    return [o0, o1, o2, o3]


def _ctw(a, num, den, sign):
    num = num % den
    if sign < 0:
        num = (den - num) % den
    if num == 0:
        return a
    if 4 * num == den:
        return (-a[1], a[0])
    if 2 * num == den:
        return (-a[0], -a[1])
    if 4 * num == 3 * den:
        return (a[1], -a[0])
    if (8 * num) % den == 0:
        r = math.sqrt(0.5)
        o = (8 * num) // den
        d = (a[0] - a[1])
        s = (a[0] + a[1])
        if o == 1:
            return (d * r, s * r)
        if o == 3:
            return (s * (-r), d * r)
        if o == 5:
            return (d * (-r), s * (-r))
        return (s * r, d * (-r))
    c = math.cos(2.0 * math.pi * num / den)
    s = math.sin(2.0 * math.pi * num / den)
    return (a[0] * c - a[1] * s, a[0] * s + a[1] * c)


def _dft8(x, sign):
    u = [_cadd(x[k], x[k + 4]) for k in range(4)]
    v = [_csub(x[k], x[k + 4]) for k in range(4)]
    ev = _dft4(u, sign)
    v1 = _ctw(v[1], 1, 8, sign)
    v3 = _ctw(v[3], 3, 8, sign)
    if sign < 0:
        t0 = (v[0][0] + v[2][1], v[0][1] - v[2][0])
        t1 = (v[0][0] - v[2][1], v[0][1] + v[2][0])
    else:
        t0 = (v[0][0] - v[2][1], v[0][1] + v[2][0])
        t1 = (v[0][0] + v[2][1], v[0][1] - v[2][0])
    t2 = _cadd(v1, v3)
    t3 = _csub(v1, v3)
    o1 = _cadd(t0, t2)
    o5 = _csub(t0, t2)
    if sign < 0:
        o3 = (t1[0] + t3[1], t1[1] - t3[0])
        o7 = (t1[0] - t3[1], t1[1] + t3[0])
    else:
        o3 = (t1[0] - t3[1], t1[1] + t3[0])
        o7 = (t1[0] + t3[1], t1[1] - t3[0])
    return [ev[0], o1, ev[1], o3, ev[2], o5, ev[3], o7]


def _gelu2a(xs):
    return xs * jnp.tanh(xs * (xs * xs + GC)) + xs


def _silu_h(hx):
    return hx * jnp.tanh(hx) + hx


def _dot(a, b):
    return jnp.dot(a, b, preferred_element_type=F32)


def _dot_nt(a, b):
    return lax.dot_general(a, b, _NT, preferred_element_type=F32)


def _rows(i, n):
    if isinstance(i, int):
        return pl.ds(i * n, n)
    return pl.ds(pl.multiple_of(i * n, n), n)


def _ds(start, n):
    if isinstance(start, int):
        return pl.ds(start, n)
    return pl.ds(pl.multiple_of(start, n), n)


def _kernel(x_hbm, wr_hbm, wi_hbm, win_hbm, wsp_hbm, bsp_hbm, wout_hbm,
            csm_hbm, cm_hbm, ctw_hbm, zero_hbm,
            out_hbm,
            xbuf, wint, csm, cmat, ctw, wbuf, wtr, wsp, wout, bspb, zsm,
            za_ref, z1_ref, y1_ref, zz_ref, xm_ref, um_ref,
            gate_ref, sbuf, obuf, bsp32,
            sem_x, sem_w, sem_sp, sem_o, *bufs):
    p1_refs, v_refs, yb_refs = bufs[0:4], bufs[4:8], bufs[8:12]
    zd_refs, lnb = bufs[12:16], bufs[16:32]
    hb_refs, tins = bufs[32:34], bufs[34:36]
    c_refs = dict(zip(("p", "11", "12", "21", "22"), bufs[36:41]))
    wa_ref, bop, zc_refs = bufs[41], bufs[42:48], bufs[48:56]
    hb_u = [r.bitcast(U32) for r in hb_refs]
    wa_u, bop_u = wa_ref.bitcast(U32), [r.bitcast(U32) for r in bop]
    lane = lax.broadcasted_iota(jnp.int32, (1, 128), 1)
    m0 = (lane & 1) == 0
    alt = jnp.where(m0, 1.0, -1.0).astype(F32)

    wint_u, csm_u, cmat_u = wint.bitcast(U32), csm.bitcast(U32), cmat.bitcast(U32)
    za_u, wout_u = za_ref.bitcast(U32), wout.bitcast(U32)
    lnb_u, tins_u = [r.bitcast(U32) for r in lnb], [r.bitcast(U32) for r in tins]
    yb_u = [r.bitcast(U32) for r in yb_refs]

    def _bf(v):
        return pltpu.bitcast(v, BF16)

    def cs(i):
        return _bf(csm_u[i])

    def x_copy(sig):
        return pltpu.make_async_copy(x_hbm.at[0, _rows(sig, 128), :],
                                     xbuf.at[_rows(sig, 128), :], sem_x.at[sig])

    def sp_copy(sig):
        return pltpu.make_async_copy(wsp_hbm.at[_rows(sig, 128), :],
                                     wsp.at[_rows(sig, 128), :], sem_sp.at[sig])

    def o_copy(sig):
        return pltpu.make_async_copy(obuf.at[_rows(sig, 128), :],
                                     out_hbm.at[0, _rows(sig, 128), :], sem_o.at[sig])

    c_win = [pltpu.make_async_copy(
        win_hbm.at[pl.ds((1 - h) * FH, FH), kd * 128:(kd + 1) * 128],
        wint.at[kd, pl.ds((1 - h) * FH, FH), :], sem_w.at[4 * h + kd])
        for h in range(2) for kd in range(4)]
    c_csf = pltpu.make_async_copy(csm_hbm.at[0:6], csm.at[0:6], sem_w.at[8])
    c_csr = pltpu.make_async_copy(csm_hbm.at[6:16], csm.at[6:16], sem_w.at[18])
    c_cm = pltpu.make_async_copy(cm_hbm, cmat, sem_w.at[9])
    c_tw = pltpu.make_async_copy(ctw_hbm, ctw, sem_w.at[10])
    c_bsp = pltpu.make_async_copy(bsp_hbm, bspb, sem_w.at[11])
    c_w = [pltpu.make_async_copy(w_hbm, wbuf.at[a], sem_w.at[12 + a])
           for a, w_hbm in enumerate((wr_hbm, wi_hbm))]
    c_wout = [pltpu.make_async_copy(wout_hbm.at[:, nt * 128:(nt + 1) * 128],
                                    wout.at[nt, 0:FH, :], sem_w.at[14 + nt])
              for nt in range(4)]
    c_zero = pltpu.make_async_copy(zero_hbm, zsm, sem_w.at[19])

    x_copy(0).start()
    c_zero.start()
    x_copy(4).start()
    for c in c_win[:4]:
        c.start()

    xm_ref[...] = jnp.zeros((128, 128), F32)
    wout[:, FH:FHP, :] = jnp.zeros((4, FHP - FH, 128), BF16)

    x_copy(0).wait()
    c_zero.wait()
    x_copy(4).wait()
    for c in c_win[4:]:
        c.start()
    x_copy(8).start()

    zero = zsm[0]
    never = jnp.full((8, 128), zero, jnp.int32) > 0

    pending = []

    def attach(p, vals, lo=0, hi=None):
        n = len(vals)
        if n == 0:
            return p
        nr = p.shape[0] // 8
        hi = nr if hi is None else hi
        at = {lo + ((u + 1) * (hi - lo)) // n - 1: vals[u] for u in range(n)}
        assert len(at) == n
        parts, r0 = [], 0
        for r in sorted(at):
            if r > r0:
                parts.append(p[r0 * 8:r * 8])
            parts.append(jnp.where(never, at[r], p[r * 8:(r + 1) * 8]))
            r0 = r + 1
        if r0 < nr:
            parts.append(p[r0 * 8:])
        return jnp.concatenate(parts, axis=0)

    def clobber(ref):
        junk = ref.shape[0] - 8
        ref[pl.ds(pl.multiple_of(junk + zero * 8, 8), 8), :] = jnp.zeros((8, 128), F32)

    def fenced(p, units, lo=0):
        return attach(p, [u() for u in units], lo)

    def drain(p, hi=None, lo=8):
        vals = [pltpu.bitcast(v, U32) for v in pending]
        del pending[:]
        return attach(p, vals, lo, hi)

    def ln_core(sig, rc, gate):
        xs = xbuf[pl.ds(sig * 128 + rc * 16, 16), :].astype(F32)
        if gate is not None:
            x00 = jnp.concatenate([jnp.where(never, gate, xs[0:8, 0:128]),
                                   jnp.where(never, gate, xs[8:16, 0:128])], axis=0)
            xs = jnp.concatenate([x00, xs[:, 128:]], axis=1)
        mu = jnp.sum(xs, axis=1, keepdims=True) * (1.0 / D)
        xc = xs - mu
        var = jnp.sum(xc * xc, axis=1, keepdims=True) * (1.0 / D)
        xn = xc * (lax.rsqrt(var + EPS) * ALPHA)
        x0, x1, x2, x3 = [xn[:, t * 128:(t + 1) * 128] for t in range(4)]
        s02 = x0 + x2
        s13 = x1 + x3
        a0 = s02 + s13
        r = pl.ds(rc * 16, 16)
        pp = x0 - x2
        q = x1 - x3
        for t, val in enumerate((a0, s02 - s13, pp, q, pp + q)):
            lnb[sig][4 + t, r, :] = val.astype(BF16)
        nyq = jnp.sum(a0 * alt, axis=1, keepdims=True)
        nyq = jnp.broadcast_to(nyq, (16, 128))
        pltpu.store(xm_ref.at[r, :], nyq,
                    mask=jnp.broadcast_to(lane == sig, (16, 128)))
        pending.append(nyq[0:8] + nyq[8:16])
        return x0, x1, x2, x3

    def ln_unit(sig, rc):
        def run(gate=None):
            for t, val in enumerate(ln_core(sig, rc, gate)):
                lnb[sig][t, pl.ds(rc * 16, 16), :] = val.astype(BF16)
        return run

    def bslot(sa):
        return 2 * (sa % 4 - 1) + sa // 4

    def lnp_unit(sa, rc):
        keep = {}

        def put(k, t, val):
            bop[bslot(sa)][2 * k + t, pl.ds(rc * 16, 16), :] = val.astype(BF16)

        def first(gate=None):
            xa = keep["xa"] = ln_core(sa, rc, gate)
            for t in range(2):
                put(1, t, xa[t])
                put(3, t, xa[2 + t] - xa[t])

        def second(gate=None):
            xa = keep["xa"]
            xb = ln_core(sa + 8, rc, gate)
            for t in range(2):
                b11, b21, b12, b22 = xa[t], xa[2 + t], xb[t], xb[2 + t]
                for k, val in ((0, b11 + b22), (2, b12 - b22), (4, b22), (5, b11 + b12),
                               (6, b21 + b22)):
                    put(k, t, val)
        return [first, second]

    _WA = {0: ((1, 0), (0, 1), 1), 1: ((0, 0), (0, 1), 1), 4: ((1, 0), (1, 1), 1),
           5: ((0, 0), (1, 0), -1), 6: ((1, 1), (0, 1), -1)}
    _WA_IDX = {k: i for i, k in enumerate(sorted(_WA))}

    def wa_unit(kind, t, ch):
        def run(gate):
            (ra, ka), (rb, kb), sign = _WA[kind]
            n = 8 if ch < 5 else 3
            au = wint_u[2 * ka + t, pl.ds(ra * (FH // 2) + ch * 64, 8 * n), :]
            au = jnp.where(jnp.full((n, 8, 128), zero, jnp.int32) > 0,
                           pltpu.bitcast(gate, U32), au.reshape(n, 8, 128))
            a = _bf(au.reshape(8 * n, 128)).astype(F32)
            b = _bf(wint_u[2 * kb + t, pl.ds(rb * (FH // 2) + ch * 64, 8 * n), :]).astype(F32)
            wa_ref[_WA_IDX[kind], t, pl.ds(ch * 128, 16 * n), :] = (
                a + b if sign > 0 else a - b).astype(BF16)
        return run

    def wa_units(kind):
        return [wa_unit(kind, t, ch) for t in range(2) for ch in range(6)]

    def release(p, units, lo=0, hi=FH // 8):
        for u, unit in enumerate(units):
            r = lo + (u * (hi - lo)) // len(units)
            unit(p[r * 8:r * 8 + 8])

    def wint_rows(r0, n):
        tiles = [wint_u[kd, pl.ds(r0 // 2, n // 2), :] for kd in range(4)]
        tiles[0] = drain(tiles[0], 30 if r0 == 0 else None)
        return jnp.concatenate([_bf(t) for t in tiles], axis=1)

    def xn_slab(sig):
        return jnp.concatenate([_bf(lnb_u[sig][t + zero]) for t in range(4)], axis=1)

    def z2_stream(sig, p):
        zd = zd_refs[sig // 4]
        c0 = s1 = s2 = None
        hist = []
        for i in range(11):
            n = 8 if i < 10 else 6
            v = p[i * 64:i * 64 + 8 * n]
            if i >= 2:
                v = jnp.concatenate([jnp.where(never, hist[i - 2][0], v[0:8]),
                                     jnp.where(never, hist[i - 2][1], v[8:16]),
                                     v[16:]], axis=0)
            y = _gelu2a(v).reshape(n, 8, 128)
            if i == 0:
                c0 = y[0]
            d = y - c0
            zd[4 * i:4 * i + n // 2] = d.reshape(n // 2, 16, 128)
            t1 = jnp.sum(d, axis=0)
            t2 = jnp.sum(d * d, axis=0)
            s1 = t1 if s1 is None else s1 + t1
            s2 = t2 if s2 is None else s2 + t2
            hist.append((s1, s2))
        ng = FH // 8
        mean_g = c0 + s1 * (1.0 / ng)
        mean = jnp.sum(mean_g, axis=0, keepdims=True) * 0.125
        dm = mean_g - mean
        m2 = s2 - s1 * s1 * (1.0 / ng) + dm * dm * float(ng)
        var = jnp.maximum(jnp.sum(m2, axis=0, keepdims=True) * (1.0 / FH), 0.0)
        rs = lax.rsqrt(var + EPS * (4.0 * ALPHA * ALPHA)) * (0.25 / ALPHA)
        rs = jnp.broadcast_to(rs, (8, 128))
        return rs, (c0 - mean) * rs

    nq1 = F1 // 16

    def put_za(kind, kt, q, val):
        za_ref[kind, kt, pl.ds(q * 16, 16), :] = val.reshape(16, 128).astype(BF16)

    def normp_units(sa, st_a, st_b):
        za_, zb_ = zd_refs[sa // 4], zd_refs[sa // 4 + 2]

        def unit(i):
            def run(gate):
                ra = jnp.where(never, gate, st_a[0])
                rb = jnp.where(never, gate, st_b[0])
                for q in (2 * i, 2 * i + 1):
                    a11 = za_[q + zero].reshape(2, 8, 128) * ra + st_a[1]
                    a12 = zb_[q + zero].reshape(2, 8, 128) * rb + st_b[1]
                    put_za(2, sa, q, a11)
                    put_za(4, sa, q, a11 + a12)
                    if q + nq1 < FH // 16:
                        a21 = za_[q + nq1 + zero].reshape(2, 8, 128) * ra + st_a[1]
                        a22 = zb_[q + nq1 + zero].reshape(2, 8, 128) * rb + st_b[1]
                        put_za(0, sa, q, a11 + a22)
                        put_za(1, sa, q, a21 + a22)
                        put_za(3, sa, q, a22)
                        put_za(5, sa, q, a21 - a11)
                        put_za(6, sa, q, a12 - a22)
                    else:
                        put_za(0, sa, q, a11)
                        put_za(6, sa, q, a12)
            return run
        return [unit(i) for i in range(11)]

    def z2_part(sig, units, extra=()):
        zd = zd_refs[sig // 4]
        p = _dot_nt(wint_rows(FH, FH), xn_slab(sig))
        release(p, units, 0, 64)
        release(p, extra)
        rs, sh = z2_stream(sig, p)
        kt = sig % 8

        def put(kind, q, val):
            put_za(kind, kt, q, val)

        def norm_unit(i):
            def run(gate):
                ri = jnp.where(never, gate, rs)
                for q in (2 * i, 2 * i + 1):
                    has2 = q + nq1 < FH // 16
                    top = zd[q + zero].reshape(2, 8, 128) * ri + sh
                    bot = (zd[q + nq1 + zero].reshape(2, 8, 128) * ri + sh) if has2 else None
                    if sig < 8:
                        zd[q] = top.reshape(16, 128)
                        put(2, q, top)
                        if has2:
                            zd[q + nq1] = bot.reshape(16, 128)
                            put(5, q, bot - top)
                    else:
                        zp = zd_refs[sig // 4 - 2]
                        a11 = zp[q + zero].reshape(2, 8, 128)
                        put(4, q, a11 + top)
                        if has2:
                            a21 = zp[q + nq1 + zero].reshape(2, 8, 128)
                            put(0, q, a11 + bot)
                            put(1, q, a21 + bot)
                            put(3, q, bot)
                            put(6, q, top - bot)
                        else:
                            put(0, q, a11)
                            put(6, q, top)
            return run
        return [norm_unit(i) for i in range(11)]

    def z1_part(sig, ln_units, norm_units, extra=()):
        p = _dot_nt(wint_rows(0, FH), xn_slab(sig))
        release(p, ln_units, 0, 64)
        release(p, norm_units, 8)
        release(p, extra)
        z1_ref[sig] = _gelu2a(p)

    def zprod(kind, sa, hard=None):
        if kind == 2:
            tiles = [wint_u[t, pl.ds(FH // 2, FH // 2), :] for t in range(2)]
        elif kind == 3:
            tiles = [wint_u[2 + t, pl.ds(0, FH // 2), :] for t in range(2)]
        else:
            tiles = [wa_u[_WA_IDX[kind] + zero, t] for t in range(2)]
        if hard is not None:
            tiles[0] = drain(tiles[0], hard[1], hard[0])
        rhs = jnp.concatenate([_bf(bop_u[bslot(sa)][2 * kind + t + zero]) for t in range(2)],
                              axis=1)
        return _dot_nt(jnp.concatenate([_bf(t) for t in tiles], axis=1), rhs)

    class Seg:
        def __init__(self, refs):
            self.refs = refs

        def get(self):
            return jnp.concatenate([r[0:FH // 2, :] for r in self.refs], axis=0)

        def put(self, v):
            for k, r in enumerate(self.refs):
                r[0:FH // 2, :] = v[k * (FH // 2):(k + 1) * (FH // 2)]
                clobber(r)

    class ZPair:
        def __init__(self, sa, k):
            self.sa = sa
            self.c11 = Seg(zc_refs[4 * k:4 * k + 2])
            self.c22 = Seg(zc_refs[4 * k + 2:4 * k + 4])

        def r1(self, lnu=(), units=(), hard=None):
            m4 = zprod(3, self.sa, hard)
            m2 = zprod(1, self.sa)
            release(m4, lnu, 0, 50)
            release(m4, units, 4)
            z1_ref[self.sa] = _gelu2a(m2 + m4)
            self.c11.put(m4)
            self.c22.put(m2)

        def r2(self, lnu=(), units=(), hard=None):
            m5 = zprod(4, self.sa, hard)
            m3 = zprod(2, self.sa)
            release(m5, lnu, 0, 50)
            release(m5, units, 4)
            self.st_b = z2_stream(self.sa + 8, m3 + m5)
            self.c11.put(self.c11.get() - m5)
            self.c22.put(m3 - self.c22.get())

        def r3(self, lnu=(), units=(), hard=None):
            m7 = zprod(6, self.sa, hard)
            m1 = zprod(0, self.sa)
            release(m7, lnu, 0, 50)
            release(m7, units, 4)
            self.st_a = z2_stream(self.sa, self.c11.get() + (m1 + m7))
            self.c22.put(self.c22.get() + m1)

        def r4(self, lnu=(), units=(), hard=None):
            m6 = zprod(5, self.sa, hard)
            release(m6, lnu, 0, 50)
            release(m6, units, 4)
            z1_ref[self.sa + 8] = _gelu2a(self.c22.get() + m6)

        def norms(self):
            return normp_units(self.sa, self.st_a, self.st_b)

    def d_fwd(j, lnu=()):
        def lhs(t, h):
            return jnp.concatenate(
                [_bf(lnb_u[j + 4 * b][t + zero, pl.ds(rc * 8, 8), :])
                 for rc in (2 * h, 2 * h + 1) for b in range(4)], axis=0)
        res = [[_dot(lhs(t, h), cs(i)) for i, t in enumerate((4, 5, 8, 6, 7))]
               for h in range(4)]
        t0, t2, k1, k2, k3 = [jnp.concatenate([res[h][i] for h in range(4)], axis=0)
                              for i in range(5)]
        release(t0, lnu, 0, 40)
        for rc in range(16):
            for c in range(2):
                g = []
                for b in range(4):
                    r0 = (rc // 2) * 64 + b * 16 + (rc % 2) * 8
                    if c == 0:
                        t0c = t0[r0:r0 + 8]
                        t2c = t2[r0:r0 + 8]
                        g.append((jnp.where(m0, t0c, t2c),
                                  pltpu.roll(jnp.where(m0, t2c, t0c), 1, 1)))
                    else:
                        k1c = k1[r0:r0 + 8]
                        g.append((k1c + k3[r0:r0 + 8], k2[r0:r0 + 8] - k1c * alt))
                o = _dft4(g, -1)
                if c == 0:
                    pending.append(o[0][1])
                r = pl.ds(j * 128 + rc * 8, 8)
                for e in range(4):
                    y1_ref[c, 0, e, r, :] = o[e][0]
                    y1_ref[c, 1, e, r, :] = o[e][1]

    for rc in range(8):
        ln_unit(0, rc)()
        ln_unit(4, rc)()
    del pending[:]
    for c in c_win[:4]:
        c.wait()
    for sig in (12, 1, 9):
        x_copy(sig).start()
    c_csf.start()

    def lns(sig):
        return [ln_unit(sig, rc) for rc in range(8)]

    class Halves:
        def __init__(self, units):
            self.units = units

        def __getitem__(self, sl):
            return [h for u in self.units[sl] for h in u]

    def lnps(sa):
        return Halves([lnp_unit(sa, rc) for rc in range(8)])

    wk = {k: wa_units(k) for k in _WA}
    norms0 = z2_part(0, [], wk[4][:6])
    norms4 = z2_part(4, [], wk[4][6:])
    for c in c_win[4:]:
        c.wait()
    x_copy(8).wait()
    rest = (5, 13, 2, 10, 6, 14, 3, 11, 7, 15)
    for sig in rest:
        x_copy(sig).start()
    z1_part(0, lns(8), norms0, wk[1][:4])
    z1_part(4, [], norms4, wk[1][4:])
    for s2 in (12, 1, 9):
        x_copy(s2).wait()
    c_csf.wait()
    for s2 in (0, 8, 2, 10):
        sp_copy(s2).start()
    for c in c_w + [c_cm, c_bsp] + c_wout + [c_tw, c_csr]:
        c.start()
    nxt = lnps(1)
    norms8 = z2_part(8, lns(12))
    z1_part(8, nxt[:3], norms8, wk[6][:4])
    d_fwd(0)
    norms12 = z2_part(12, nxt[3:], wk[6][4:6])
    z1_part(12, [], norms12, wk[6][6:])
    for s2 in rest:
        x_copy(s2).wait()
    prev = []
    lb = lnps(5)
    for j in range(1, 4):
        za_p, zb_p = ZPair(j, 0), ZPair(j + 4, 1)
        one = j == 1
        nxa = lnps(j + 1) if j < 3 else Halves([])
        nxb = lnps(j + 5) if j < 3 else Halves([])
        k = 0 if one else 2
        za_p.r1(lb[k:k + 4] if not one else lb[0:5], wk[0][:6] if one else [])
        za_p.r2(lb[k + 4:] if not one else lb[5:], wk[0][6:] if one else prev[:4])
        za_p.r3((), prev[4:], (8, 30))
        zb_p.r1(nxa[:1], za_p.norms())
        d_fwd(j, nxa[1:3])
        zb_p.r2(nxa[3:5], wk[5][:6] if one else [], (8, 40))
        zb_p.r3(nxa[5:], wk[5][6:] if one else [])
        prev = zb_p.norms()
        za_p.r4(nxb[:2], prev if j == 3 else [], (8, 30))
        zb_p.r4()
        lb = nxb

    _RHS = {0: ((0, 0, 1), (1, 1, 1)), 1: ((0, 0, 1),), 2: ((1, 0, 1), (1, 1, -1)),
            3: ((0, 1, 1), (0, 0, -1)), 4: ((1, 1, 1),), 5: ((0, 0, 1), (1, 0, 1)),
            6: ((0, 1, 1), (1, 1, 1))}
    _OUT = {0: (("11", 1), ("22", 1)), 1: (("21", 1), ("22", -1)),
            2: (("12", 1), ("22", 1)), 3: (("11", 1), ("21", 1)),
            4: (("11", -1), ("12", 1)), 5: (("22", 1),), 6: (("11", 1),)}

    class Pair:
        def __init__(self, s1):
            self.s = (s1, s1 + 8)
            self.c = {}
            self.neg = set()

        def p(self, m, kp, units=(), lo=0, hard=False):
            rows = F2 if m in (1, 3, 5) else F1
            tiles = [za_u[m, 4 * kp + t, 0:rows // 2, :] for t in range(4)]
            if hard:
                tiles[0] = drain(tiles[0], 20, 2)
            lhs = jnp.concatenate([_bf(t) for t in tiles], axis=1)
            blk = [wsp[_rows(self.s[th], 128), pl.ds(sh * 1024 + kp * 512, 512)]
                   for th, sh, _ in _RHS[m]]
            if len(blk) == 1:
                rhs = blk[0]
            else:
                a, b = blk[0].astype(F32), blk[1].astype(F32)
                rhs = (a + b if _RHS[m][1][2] > 0 else a - b).astype(BF16)
            p = _dot_nt(lhs, rhs)
            self.mid = p[200:208]
            p = fenced(p, list(units), lo)
            if kp == 0:
                c_refs["p"][0:rows, :] = p
                clobber(c_refs["p"])
                return
            p = c_refs["p"][0:rows, :] + p
            for name, sign in _OUT[m]:
                ref = c_refs[name]
                n = F1 if name[0] == "1" else F2
                k = min(n, rows)
                if name in self.neg:
                    assert sign > 0 and k == n
                    self.neg.remove(name)
                    ref[0:k, :] = p[0:k] - ref[0:k, :]
                elif name not in self.c:
                    if sign < 0:
                        self.neg.add(name)
                    ref[0:k, :] = p[0:k]
                    if k < n:
                        ref[k:n, :] = jnp.zeros((n - k, 128), F32)
                elif sign > 0:
                    ref[0:k, :] = ref[0:k, :] + p[0:k]
                else:
                    ref[0:k, :] = ref[0:k, :] - p[0:k]
                self.c[name] = True
                clobber(ref)

        def both(self, m, u0=(), u1=()):
            self.p(m, 0, u0)
            self.p(m, 1, u1)

        def acc(self, which):
            return c_acc(which)

    def c_acc(which):
        a, b = ("11", "21") if which == 0 else ("12", "22")
        return jnp.concatenate([c_refs[a][0:F1, :], c_refs[b][0:F2, :]], axis=0)

    def h_tiles(sig, acc, slot):
        bias = bsp32[pl.ds(sig, 1), :]
        for t in range(6):
            n = 128 if t < 5 else FH - 640
            ht = z1_ref[sig, pl.ds(t * 128, n), :] * (acc[t * 128:t * 128 + n] + bias)
            if n < 128:
                ht = jnp.concatenate([ht, jnp.zeros((128 - n, 128), F32)], axis=0)
            ht = ht.astype(BF16).T
            hb_refs[slot][t] = ht
            pending.append(pltpu.bitcast(ht[112:128], F32))

    def small(slot, after=None, units=()):
        tiles = [hb_u[slot][t + zero] for t in range(6)]
        if after is not None:
            tiles[0] = attach(tiles[0], [pltpu.bitcast(after.mid, U32)], 0, 1)
        h = jnp.concatenate([_bf(t) for t in tiles], axis=1)
        wo = jnp.concatenate([_bf(wout_u[nt]) for nt in range(4)], axis=1)
        bo = _dot(h, wo)
        if units:
            n = len(units)
            bo = jnp.concatenate(
                [fenced(bo[:, nt * 128:(nt + 1) * 128], units[nt * n // 4:(nt + 1) * n // 4])
                 for nt in range(4)], axis=1)
        return _silu_h(bo)

    def f_unit(c, e, rc):
        def run():
            xs = []
            for a in range(8):
                r = pl.ds(a * 64 + rc * 8, 8)
                xs.append(_ctw((y1_ref[c + zero, 0, e, r, :], y1_ref[c + zero, 1, e, r, :]),
                               a * e, 32, -1))
            o = _dft8(xs, -1)
            for cc in range(8):
                p1_refs[e][c, cc, pl.ds(rc * 8, 8), :] = o[cc][0]
                p1_refs[e][c, cc, pl.ds(64 + rc * 8, 8), :] = o[cc][1]
            return o[7][1]
        return run

    def f_units(e):
        return [f_unit(c, e, rc) for c in range(2) for rc in range(8)]

    def w_unit(a, kb):
        def run():
            wt = pltpu.bitcast(wbuf[a, 0:256, kb * 128:(kb + 1) * 128], U32).T
            for h in range(4):
                wtr[a, pl.ds((4 * kb + h) * WP, 32), :] = wt[h * 32:(h + 1) * 32]
            return pltpu.bitcast(wt[120:128], F32)
        return run

    def mid1(e):
        for cc in range(8):
            klo = e + 4 * cc
            wru = wtr[0, pl.ds(klo, 64, stride=WP), :]
            wiu = wtr[1, pl.ds(klo, 64, stride=WP), :]
            for c in range(2):
                if c == 0:
                    wr = pltpu.bitcast(wru << 16, F32)
                    wi = pltpu.bitcast(wiu << 16, F32)
                else:
                    wr = pltpu.bitcast(wru & jnp.uint32(0xFFFF0000), F32)
                    wi = pltpu.bitcast(wiu & jnp.uint32(0xFFFF0000), F32)
                xh = _dot(_bf(cmat_u[0, klo]), p1_refs[e][c + zero, cc].astype(BF16))
                xr, xi = xh[0:64], xh[64:128]
                yb_refs[e][c, cc, 0:64, :] = (xr * wr - xi * wi).astype(BF16)
                yb_refs[e][c, cc, 64:128, :] = (xr * wi + xi * wr).astype(BF16)

    def mid2(e, units=()):
        n = len(units)
        for cc in range(8):
            klo = e + 4 * cc
            for c in range(2):
                k = 2 * cc + c
                v = _dot(_bf(cmat_u[1, klo]), _bf(yb_u[e][c + zero, cc]))
                v_refs[e][c, cc] = fenced(v, units[k * n // 16:(k + 1) * n // 16])

    def i_unit(c, e, rc):
        def run():
            xs = []
            for cc in range(8):
                xs.append((v_refs[e][c + zero, cc, pl.ds(rc * 8, 8), :],
                           v_refs[e][c + zero, cc, pl.ds(64 + rc * 8, 8), :]))
            o = _dft8(xs, +1)
            for a in range(8):
                t = _ctw(o[a], a * e, 32, +1)
                r = pl.ds(a * 64 + rc * 8, 8)
                zz_ref[c, 0, e, r, :] = t[0]
                zz_ref[c, 1, e, r, :] = t[1]
            return t[1]
        return run

    def i_units(e):
        return [i_unit(c, e, rc) for c in range(2) for rc in range(8)]

    nq = {}

    def nyq0():
        twc, tws = ctw[0], ctw[1]
        aa = _dot_nt(_bf(csm_u[12, 0:16, :]), xm_ref[...].astype(BF16))
        ar, ai = aa[0:16], aa[16:32]
        nq[0] = jnp.concatenate([ar * twc + ai * tws, ai * twc - ar * tws], axis=0)

    def nyq1():
        l16 = lax.broadcasted_iota(jnp.int32, (16, 128), 1)
        r16 = lax.broadcasted_iota(jnp.int32, (16, 128), 0)
        idx = 16 * (l16 & 7) + r16
        grp = l16 >> 3
        wn = []
        for a in range(2):
            wrow = wbuf[a, 256:257, :].astype(F32)
            acc = jnp.zeros((16, 128), F32)
            for ka in range(16):
                rowb = jnp.broadcast_to(wrow[:, ka * 128:(ka + 1) * 128], (16, 128))
                acc = jnp.where(grp == ka, jnp.take_along_axis(rowb, idx, axis=1), acc)
            wn.append(acc)
        cs128 = jnp.concatenate([cs(14), cs(15)], axis=1)
        p = _dot(nq[0].astype(BF16), cs128)
        xr = p[0:16, 0:128] + p[16:32, 128:256]
        xi = p[16:32, 0:128] - p[0:16, 128:256]
        nq[1] = jnp.concatenate([xr * wn[0] - xi * wn[1], xr * wn[1] + xi * wn[0]], axis=0)

    def nyq2():
        twc, tws = ctw[0], ctw[1]
        cs128 = jnp.concatenate([cs(14), cs(15)], axis=1)
        p = _dot(nq[1].astype(BF16), cs128)
        vr = p[0:16, 0:128] - p[16:32, 128:256]
        vi = p[16:32, 0:128] + p[0:16, 128:256]
        nq[2] = jnp.concatenate([vr * twc - vi * tws, vi * twc + vr * tws,
                                 jnp.zeros((96, 128), F32)], axis=0)

    def nyq3():
        um_ref[...] = _dot(nq[2].T.astype(BF16), cs(13))

    for c in (c_wout + c_w + [c_cm, c_tw, c_bsp, c_csr]
              + [sp_copy(sig) for sig in (0, 8, 2, 10)]):
        c.wait()
    for sig in (4, 12, 1, 9, 5, 13, 6, 14, 3, 11, 7, 15):
        sp_copy(sig).start()
    bsp32[...] = bspb[...].astype(F32) * (0.25 / ALPHA)
    wu = [w_unit(a, kb) for kb in range(NS) for a in range(2)]
    fu = [f_units(e) for e in range(4)]
    iu = [i_units(e) for e in range(4)]
    pa, pb = Pair(0), Pair(2)

    def mix(a, b):
        out = []
        for k in range(max(len(a), len(b))):
            out += a[k:k + 1] + b[k:k + 1]
        return out

    pa.p(3, 0, mix(fu[0][0:4], wu[0:4]))
    pa.p(3, 1, mix(fu[0][4:8], wu[4:8]))
    pa.p(1, 0, mix(fu[0][8:16], wu[8:14]))
    pa.p(1, 1, mix(fu[1][0:6], wu[14:20]))
    pa.p(6, 0, mix(fu[1][6:9], wu[20:26]))
    pa.p(6, 1, mix(fu[1][9:12], wu[26:32]))
    nyq0()
    pa.p(4, 0, fu[1][12:16])
    mid1(0)
    pa.p(4, 1, fu[2][0:6])
    mid2(0, fu[2][6:16])
    pa.p(0, 0, iu[0][0:4])
    mid1(1)
    pa.p(0, 1, iu[0][4:8])
    h_tiles(0, pa.acc(0), 0)
    nyq1()
    mid2(1, iu[0][8:16] + fu[3][0:6])
    pa.p(2, 0, fu[3][6:9], 0, True)
    gate_ref[0] = small(0, pa, fu[3][9:16] + iu[1][0:8])
    pa.p(2, 1, iu[1][8:12])
    mid1(2)
    pa.p(5, 0, iu[1][12:16])
    mid2(2)
    nyq2()
    pa.p(5, 1, iu[2][0:4])
    h_tiles(8, pa.acc(1), 1)
    mid1(3)
    pb.p(3, 0, iu[2][4:8], 0, True)
    gate_ref[1] = small(1, pb, iu[2][8:16])
    mid2(3)
    nyq3()
    pb.p(3, 1, iu[3][0:4])
    pb.both(1, iu[3][4:12], iu[3][12:16])
    pb.both(6)
    pb.both(4)
    pb.both(0)
    h_tiles(2, pb.acc(0), 0)
    pb.p(2, 0)
    pb.p(2, 1, hard=True)
    gate_ref[2] = small(0, pb)
    pb.both(5)
    sbuf[5] = jnp.zeros((128, D), F32)

    def emit(sig, rc, sv, g, dst=None):
        r = _ds(sig * 128 + rc * 16, 16)
        ro = r if dst is None else _ds(dst * 128 + rc * 16, 16)
        obuf[ro, :] = (xbuf[r, :].astype(F32) + sv * g).astype(BF16)

    def finish(sig, slot, g, dst=None):
        for rc in range(8):
            emit(sig, rc, sbuf[slot + zero, pl.ds(rc * 16, 16), :],
                 g[rc * 16:(rc + 1) * 16], dst)

    def r_units(j, tb):
        tin = tins[tb]

        def r_unit(c, rc):
            def run():
                r = _ds(j * 128 + rc * 16, 16)
                u = _dft4([(zz_ref[c, 0, e, r, :], zz_ref[c, 1, e, r, :])
                           for e in range(4)], +1)
                for b in range(4):
                    ro = pl.ds(rc * 64 + b * 16, 16)
                    re, im = u[b]
                    if c == 0:
                        nq_col = pltpu.roll(um_ref[pl.ds(rc * 16, 16), :],
                                            (128 - 4 * b - j) % 128, 1)
                        ip = pltpu.roll(jnp.where(lane == 0, nq_col, im), 127, 1)
                        tin[0, ro, :] = jnp.where(m0, re, ip).astype(BF16)
                        tin[1, ro, :] = jnp.where(m0, ip, re).astype(BF16)
                    else:
                        im = im * alt
                        tin[2, ro, :] = (re + im).astype(BF16)
                        tin[3, ro, :] = re.astype(BF16)
                        tin[4, ro, :] = im.astype(BF16)
                return ip[8:16] if c == 0 else u[3][1][8:16]
            return run
        return [r_unit(c, rc) for rc in range(8) for c in range(2)]

    def d_inv(j, tb, sink):
        tin_u = tins_u[tb]
        res = [[_dot(_bf(tin_u[i + zero, pl.ds(h * 64, 64), :]), cs(6 + i)) for i in range(5)]
               for h in range(4)]
        b0, b2, k1, k2, k3 = [jnp.concatenate([res[h][i] for h in range(4)], axis=0)
                              for i in range(5)]
        for rc in range(8):
            for b in range(4):
                r0 = rc * 64 + b * 16
                b0c = b0[r0:r0 + 16]
                b2c = b2[r0:r0 + 16]
                pc = k1[r0:r0 + 16] + k3[r0:r0 + 16]
                qc = k1[r0:r0 + 16] + k2[r0:r0 + 16]
                e02 = b0c + b2c
                o02 = b0c - b2c
                sink(b, rc, jnp.concatenate([e02 + pc, o02 - qc, e02 - pc, o02 + qc], axis=1))

    def phase3(i, carry):
        j0, j1 = 2 * i, 2 * i + 1
        for d in (4, 12, 1, 9, 5, 13):
            sp_copy(j0 + d).wait()

        def sink0(b, rc, sv):
            if b % 2 == 0:
                emit(j0 + 4 * b, rc, sv, gate_ref[j0 + b // 2, pl.ds(rc * 16, 16), :])
            else:
                sbuf[b // 2, pl.ds(rc * 16, 16), :] = sv

        def sink1(b, rc, sv):
            sbuf[2 + b, pl.ds(rc * 16, 16), :] = sv

        def done(sig, slot, g):
            finish(sig, slot, g)
            o_copy(sig).start()

        first = i == 0
        car = jnp.where(first, 10, 13)
        qa, qb, qc = Pair(j0 + 4), Pair(j1), Pair(j1 + 4)
        r0, r1 = r_units(j0, 0), r_units(j1, 1)
        h_tiles(car, c_acc(1), 1)
        qa.p(3, 0, r0[:8])
        qa.p(3, 1, r0[8:], 0, True)
        g = small(1, qa)
        gate_ref[jnp.where(first, 3, 4)] = g
        finish(car, 5, g, jnp.where(first, NS, car))
        qa.p(1, 0)
        d_inv(j0, 0, sink0)
        o_copy(j0).start()
        o_copy(j0 + 8).start()
        qa.p(1, 1)
        qa.both(6)
        qa.both(4)
        qa.both(0)
        h_tiles(j0 + 4, qa.acc(0), 0)
        qa.p(2, 0)
        qa.p(2, 1, hard=True)
        done(j0 + 4, 0, small(0, qa))
        qa.both(5, r1[:8], r1[8:])
        h_tiles(j0 + 12, qa.acc(1), 1)
        qb.p(3, 0)
        qb.p(3, 1, hard=True)
        done(j0 + 12, 1, small(1, qb))
        d_inv(j1, 1, sink1)
        qb.both(1)
        qb.both(6)
        qb.both(4)
        qb.both(0)
        h_tiles(j1, qb.acc(0), 0)
        qb.p(2, 0)
        qb.p(2, 1, hard=True)
        done(j1, 2, small(0, qb))
        qb.both(5)
        h_tiles(j1 + 8, qb.acc(1), 1)
        qc.p(3, 0)
        qc.p(3, 1, hard=True)
        done(j1 + 8, 4, small(1, qc))
        qc.both(1)
        qc.both(6)
        qc.both(4)
        qc.both(0)
        h_tiles(j1 + 4, qc.acc(0), 0)
        qc.p(2, 0)
        qc.p(2, 1, hard=True)
        done(j1 + 4, 3, small(0, qc))
        qc.both(5)

        @pl.when(i > 0)
        def _():
            o_copy(13).start()
        return carry

    lax.fori_loop(0, 2, phase3, 0)
    ht = z1_ref[NS - 1] * (c_acc(1) + bsp32[NS - 1:NS, :])
    ht = jnp.concatenate([ht, jnp.zeros((FHP - FH, 128), F32)], axis=0).astype(BF16)
    wo = jnp.concatenate([_bf(wout_u[nt]) for nt in range(4)], axis=1)
    finish(NS - 1, 5, _silu_h(_dot(ht.T, wo)))
    o_copy(NS - 1).start()
    for sig in range(NS):
        o_copy(sig).wait()


@jax.jit
def pallas_recurrent_scan__spectral_gfnet__mixer_gmlp__prompt_kernel(
    A_x: jax.Array,
    A_w_r: jax.Array,
    A_w_i: jax.Array,
    B_x: jax.Array,
    B_w_in: jax.Array,
    B_w_sp: jax.Array,
    B_b_sp: jax.Array,
    B_w_out: jax.Array,
):
    del B_x
    small, cm, tw = _tables()
    csm = jnp.asarray(small, dtype=BF16)
    cmat = jnp.asarray(cm, dtype=BF16)
    ctw = jnp.asarray(tw, dtype=F32)
    zero = np.zeros((1,), np.int32)
    hbm = pl.BlockSpec(memory_space=pltpu.HBM)
    scratch = [
        pltpu.VMEM((S, D), BF16),
        pltpu.VMEM((4, F, 128), BF16),
        pltpu.VMEM((16, 128, 128), BF16),
        pltpu.VMEM((2, 32, 128, 128), BF16),
        pltpu.VMEM((2, 16, 128), F32),
        pltpu.VMEM((2, D // 2 + 1, S), BF16),
        pltpu.VMEM((2, 64 * WP, 128), U32),
        pltpu.VMEM((S, S), BF16),
        pltpu.VMEM((4, FHP, 128), BF16),
        pltpu.VMEM((NS, 128), BF16),
        pltpu.SMEM((1,), jnp.int32),
        pltpu.VMEM((7, 8, F1, 128), BF16),
        pltpu.VMEM((NS, FH, 128), F32),
        pltpu.VMEM((2, 2, 4, 512, 128), F32),
        pltpu.VMEM((2, 2, 4, 512, 128), F32),
        pltpu.VMEM((128, 128), F32),
        pltpu.VMEM((128, 128), F32),
        pltpu.VMEM((5, 128, D), F32),
        pltpu.VMEM((6, 128, D), F32),
        pltpu.VMEM((S + 128, D), BF16),
        pltpu.VMEM((NS, 128), F32),
        pltpu.SemaphoreType.DMA((NS,)),
        pltpu.SemaphoreType.DMA((20,)),
        pltpu.SemaphoreType.DMA((NS,)),
        pltpu.SemaphoreType.DMA((NS,)),
    ]
    scratch += [pltpu.VMEM((2, 8, 128, 128), F32)] * 8
    scratch += [pltpu.VMEM((2, 8, 128, 128), BF16)] * 4
    scratch += [pltpu.VMEM((FH // 16, 16, 128), F32)] * 4
    scratch += [pltpu.VMEM((9, 128, 128), BF16)] * NS
    scratch += [pltpu.VMEM((6, 128, 128), BF16)] * 2
    scratch += [pltpu.VMEM((5, 512, 128), BF16)] * 2
    scratch += [pltpu.VMEM((F1 + 8, 128), F32)] * 5
    scratch += [pltpu.VMEM((5, 2, FH, 128), BF16)]
    scratch += [pltpu.VMEM((14, 128, 128), BF16)] * 6
    scratch += [pltpu.VMEM((FH // 2 + 8, 128), F32)] * 8
    return pl.pallas_call(
        _kernel,
        out_shape=jax.ShapeDtypeStruct((1, S, D), BF16),
        in_specs=[hbm] * 11,
        out_specs=hbm,
        scratch_shapes=scratch,
        compiler_params=pltpu.CompilerParams(vmem_limit_bytes=100 * 1024 * 1024),
    )(A_x, A_w_r.T, A_w_i.T, B_w_in.T, B_w_sp, B_b_sp.reshape(NS, 128), B_w_out,
      csm, cmat, ctw, zero)
```
